```python
import jax
import jax.numpy as jnp

def _softmax(x, axis=-1):
    return jax.nn.softmax(x, axis=axis)
def _gelu(x):
    return jax.nn.gelu(x, approximate=True)
def _silu(x):
    return jax.nn.silu(x)
def _sigmoid(x):
    return jax.nn.sigmoid(x)
def _layernorm(x, axis=-1, eps=1e-5):
    m = jnp.mean(x, axis=axis, keepdims=True)
    v = jnp.var(x, axis=axis, keepdims=True)
    return (x - m) / jnp.sqrt(v + eps)
def _scatter_add(tgt, idx, src, axis=0):
    return tgt.at[idx].add(src)
def _segment_sum(src, seg, n):
    return jax.ops.segment_sum(src, seg, n)
class _Rng:
    def __init__(self, key):
        self._k = key
    def _next(self):
        self._k, sub = jax.random.split(self._k)
        return sub
    def normal(self, shape):
        return jax.random.normal(self._next(), shape, dtype=jnp.bfloat16)
    def randint(self, lo, hi, shape):
        return jax.random.randint(self._next(), shape, lo, hi, dtype=jnp.int32)
    def uniform(self, shape, lo=0.0, hi=1.0):
        return jax.random.uniform(self._next(), shape, jnp.bfloat16, lo, hi)
    def permutation(self, n):
        return jax.random.permutation(self._next(), n)


kernel_name = 'parallel_sum__sliding_block_cached__moe_arch_mod__decode'

def setup_inputs():
    _rng = _Rng(jax.random.key(int.from_bytes(__import__("os").urandom(4), "little")))
    _w = (lambda a: (lambda t: t.astype(jnp.bfloat16) if jnp.issubdtype(t.dtype, jnp.floating) else t)(jnp.asarray(a)))
    def _A_setup():
        B, Sq, D = 1, 1, 512
        Hq, Hkv, Sk, Dh = 32, 8, 65536, 128
        assert Hq % Hkv == 0, (Hq, Hkv)
        return {
            "x": _w((lambda *s: _rng.normal(s) * 0.05)(B, Sq, D)),
            "k_cache": _w((lambda *s: _rng.normal(s) * 0.05)(B, Hkv, Sk, Dh)),
            "v_cache": _w((lambda *s: _rng.normal(s) * 0.05)(B, Hkv, Sk, Dh)),
            "wq": _w((lambda *s: _rng.normal(s) * 0.05)(D, Hq * Dh) * (D ** -0.5)),
            "wo": _w((lambda *s: _rng.normal(s) * 0.05)(Hq * Dh, D) * ((Hq * Dh) ** -0.5)),
        }
    _A_in = _A_setup()

    def _B_setup():
        B, S, D, F, C = 1, 1, 512, 1792, 1
        return {
            "x": _w((lambda *s: _rng.normal(s) * 0.05)(B, S, D)),
            "w_r": _w((lambda *s: _rng.normal(s) * 0.05)(D)),
            "w_gate": _w((lambda *s: _rng.normal(s) * 0.05)(D, F)),
            "w_up": _w((lambda *s: _rng.normal(s) * 0.05)(D, F)),
            "w_down": _w((lambda *s: _rng.normal(s) * 0.05)(F, D)),
        }
    _B_in = _B_setup()

    return {
        "A_x": _A_in["x"],
        "A_k_cache": _A_in["k_cache"],
        "A_v_cache": _A_in["v_cache"],
        "A_wq": _A_in["wq"],
        "A_wo": _A_in["wo"],
        "B_x": _B_in["x"],
        "B_w_r": _B_in["w_r"],
        "B_w_gate": _B_in["w_gate"],
        "B_w_up": _B_in["w_up"],
        "B_w_down": _B_in["w_down"],
    }

def reference(A_x, A_k_cache, A_v_cache, A_wq, A_wo, B_x, B_w_r, B_w_gate, B_w_up, B_w_down):
    def _A_ref(x, k_cache, v_cache, wq, wo):
        B, Sq, D = x.shape
        Hq, Dh = 32, 128
        Hkv, Sk = k_cache.shape[1], k_cache.shape[2]
        W = min(4096, max(256, Sk // 4))
        rep = Hq // Hkv
        q = (lambda x, *d: x.transpose(*d))((x @ wq).reshape(B, Sq, Hq, Dh), 0, 2, 1, 3)
        k = jnp.repeat(k_cache[:, :, Sk - W:, :], rep, axis=1)
        v = jnp.repeat(v_cache[:, :, Sk - W:, :], rep, axis=1)
        scores = jnp.einsum("bhqd,bhkd->bhqk", q, k) * (Dh ** -0.5)
        p = _softmax(scores, axis=-1)
        o = jnp.einsum("bhqk,bhkd->bhqd", p, v)
        return (lambda x, *d: x.transpose(*d))(o, 0, 2, 1, 3).reshape(B, Sq, Hq * Dh) @ wo

    def _B_ref(x, w_r, w_gate, w_up, w_down):
        B, S, D = x.shape
        C = 1
        r = x @ w_r
        idx = jnp.argsort(-r, axis=-1)[:, :C]
        idx_e = jnp.repeat(idx.reshape(B, C, 1), D, axis=2)
        x_sel = jnp.take_along_axis(x, idx_e, axis=1)
        g = _silu(x_sel @ w_gate)
        u = x_sel @ w_up
        y = (g * u) @ w_down
        r_sel = _sigmoid(jnp.take_along_axis(r, idx, axis=1))
        y = y * r_sel.reshape(B, C, 1)
        b_off = (jnp.arange(B) * S).reshape(B, 1)
        flat_idx = (idx + b_off).reshape(B * C)
        zero = (x * 0.0).reshape(B * S, D)
        upd = _scatter_add(zero, flat_idx, y.reshape(B * C, D), axis=0)
        return x + upd.reshape(B, S, D)

    x = A_x
    xn = _layernorm(x, axis=-1)
    return x + _A_ref(xn, A_k_cache, A_v_cache, A_wq, A_wo) + _B_ref(xn, B_w_r, B_w_gate, B_w_up, B_w_down)
```

```python
import jax
import jax.numpy as jnp
from jax import lax
import jax.experimental.pallas as pl
import jax.experimental.pallas.tpu as pltpu

HQ, DH = 32, 128
F32 = jnp.float32
BF16 = jnp.bfloat16
NT = (((1,), (1,)), ((), ()))

WQ_CH = 4
WO_CH = 4
WD_CH = (768, 768, 256)
M = 8


def _kernel(x_hbm, k_hbm, v_hbm, wq_hbm, wo_hbm, wr_hbm, wg_hbm, wu_hbm, wd_hbm, out_ref,
            x_v, wr_v, wq_v, k_v, v_v, wo_v, wg_v, wu_v, wd_v, q_s, o_s, sems):
    hkv, sk = k_hbm.shape[1], k_hbm.shape[2]
    W = k_v.shape[1]
    D = x_v.shape[-1]
    rep = HQ // hkv
    wq_rows = D // WQ_CH
    wo_rows = (HQ * DH) // WO_CH
    wd_off = [sum(WD_CH[:i]) for i in range(len(WD_CH))]
    S_X, S_WR, S_WQ = 0, 1, 2
    S_K = S_WQ + WQ_CH
    S_V = S_K + hkv
    S_WO = S_V + hkv
    S_WG = S_WO + WO_CH
    S_WU = S_WG + 1
    S_WD = S_WU + 1

    def rows_copy(src, dst, off, n, s):
        return pltpu.make_async_copy(src.at[pl.ds(off, n)], dst.at[pl.ds(off, n)], sems.at[s])

    def cp_x():
        return pltpu.make_async_copy(x_hbm, x_v, sems.at[S_X])

    def cp_wr():
        return pltpu.make_async_copy(wr_hbm, wr_v, sems.at[S_WR])

    def cp_wq(c):
        return rows_copy(wq_hbm, wq_v, c * wq_rows, wq_rows, S_WQ + c)

    def cp_k(h):
        return pltpu.make_async_copy(k_hbm.at[0, h, pl.ds(sk - W, W)], k_v.at[h], sems.at[S_K + h])

    def cp_v(h):
        return pltpu.make_async_copy(v_hbm.at[0, h, pl.ds(sk - W, W)], v_v.at[h], sems.at[S_V + h])

    def cp_wo(c):
        return rows_copy(wo_hbm, wo_v, c * wo_rows, wo_rows, S_WO + c)

    def cp_wg():
        return pltpu.make_async_copy(wg_hbm, wg_v, sems.at[S_WG])

    def cp_wu():
        return pltpu.make_async_copy(wu_hbm, wu_v, sems.at[S_WU])

    def cp_wd(c):
        return rows_copy(wd_hbm, wd_v, wd_off[c], WD_CH[c], S_WD + c)

    cp_wq(0).start()
    cp_x().start()
    cp_wr().start()
    for c in range(1, WQ_CH):
        cp_wq(c).start()
    for h in range(hkv):
        cp_k(h).start()
        cp_v(h).start()
    cp_wg().start()
    cp_wu().start()
    for c in range(WO_CH):
        cp_wo(c).start()
    for c in range(len(WD_CH)):
        cp_wd(c).start()

    cp_x().wait()
    x = x_v[0].astype(F32)
    mu = jnp.mean(x, axis=-1, keepdims=True)
    xc = x - mu
    var = jnp.mean(xc * xc, axis=-1, keepdims=True)
    xn = xc / jnp.sqrt(var + 1e-5)
    xb = jnp.broadcast_to(xn, (M, D)).astype(BF16)

    cp_wr().wait()
    wr = wr_v[...].astype(F32).reshape(1, D)
    r = jnp.sum(xn * wr, axis=-1, keepdims=True)
    gate = jax.nn.sigmoid(r)

    q = None
    for c in range(WQ_CH):
        cp_wq(c).wait()
        part = jnp.dot(xb[:, c * wq_rows:(c + 1) * wq_rows], wq_v[c * wq_rows:(c + 1) * wq_rows, :],
                       preferred_element_type=F32)
        q = part if q is None else q + part
    q = q * (DH ** -0.5)
    row = lax.broadcasted_iota(jnp.int32, (M, DH), 0)
    for h in range(hkv):
        qh = q[:, (h * rep) * DH:(h * rep + 1) * DH]
        for j in range(1, rep):
            qh = jnp.where(row == j, q[:, (h * rep + j) * DH:(h * rep + j + 1) * DH], qh)
        q_s[h] = qh

    def head(h, carry):
        cp_k(h).wait()
        qh = q_s[h].astype(BF16)
        s = lax.dot_general(qh, k_v[h], NT, preferred_element_type=F32)
        m = jnp.max(s, axis=-1, keepdims=True)
        p = jnp.exp(s - m)
        l = jnp.sum(p, axis=-1, keepdims=True)
        cp_v(h).wait()
        o = jnp.dot(p.astype(BF16), v_v[h], preferred_element_type=F32)
        o_s[h] = o / l
        return carry
    lax.fori_loop(0, hkv, head, 0)

    cp_wg().wait()
    g = jnp.dot(xb, wg_v[...], preferred_element_type=F32)
    cp_wu().wait()
    u = jnp.dot(xb, wu_v[...], preferred_element_type=F32)
    hh = (g * jax.nn.sigmoid(g) * u).astype(BF16)

    pieces = []
    for h in range(hkv):
        oh = o_s[h]
        for j in range(rep):
            pieces.append(jnp.where(row == j, oh, 0.0).astype(BF16))
    obd = jnp.concatenate(pieces, axis=1)
    acc = None
    for c in range(WO_CH):
        cp_wo(c).wait()
        part = jnp.dot(obd[:, c * wo_rows:(c + 1) * wo_rows], wo_v[c * wo_rows:(c + 1) * wo_rows, :],
                       preferred_element_type=F32)
        acc = part if acc is None else acc + part
    attn = jnp.sum(acc, axis=0, keepdims=True)
    base = x + xn + attn

    y = None
    for c in range(len(WD_CH)):
        cp_wd(c).wait()
        part = jnp.dot(hh[:, wd_off[c]:wd_off[c] + WD_CH[c]], wd_v[wd_off[c]:wd_off[c] + WD_CH[c], :],
                       preferred_element_type=F32)
        y = part if y is None else y + part
    out_ref[0] = (base + y[0:1, :] * gate).astype(out_ref.dtype)


@jax.jit
def pallas_parallel_sum__sliding_block_cached__moe_arch_mod__decode_kernel(
    A_x: jax.Array,
    A_k_cache: jax.Array,
    A_v_cache: jax.Array,
    A_wq: jax.Array,
    A_wo: jax.Array,
    B_x: jax.Array,
    B_w_r: jax.Array,
    B_w_gate: jax.Array,
    B_w_up: jax.Array,
    B_w_down: jax.Array,
):
    del B_x
    hkv, sk = A_k_cache.shape[1], A_k_cache.shape[2]
    W = min(4096, max(256, sk // 4))
    nsem = 2 + WQ_CH + 2 * hkv + WO_CH + 2 + len(WD_CH)
    anyspec = pl.BlockSpec(memory_space=pl.ANY)
    return pl.pallas_call(
        _kernel,
        out_shape=jax.ShapeDtypeStruct(A_x.shape, A_x.dtype),
        in_specs=[anyspec] * 9,
        out_specs=pl.BlockSpec(memory_space=pltpu.VMEM),
        scratch_shapes=[
            pltpu.VMEM(A_x.shape, BF16), pltpu.VMEM(B_w_r.shape, BF16),
            pltpu.VMEM(A_wq.shape, BF16),
            pltpu.VMEM((hkv, W, DH), BF16), pltpu.VMEM((hkv, W, DH), BF16),
            pltpu.VMEM(A_wo.shape, BF16),
            pltpu.VMEM(B_w_gate.shape, BF16), pltpu.VMEM(B_w_up.shape, BF16),
            pltpu.VMEM(B_w_down.shape, BF16),
            pltpu.VMEM((hkv, M, DH), F32), pltpu.VMEM((hkv, M, DH), F32),
            pltpu.SemaphoreType.DMA((nsem,)),
        ],
        compiler_params=pltpu.CompilerParams(
            vmem_limit_bytes=48 * 1024 * 1024,
            disable_semaphore_checks=True,
        ),
    )(A_x, A_k_cache, A_v_cache, A_wq, A_wo, B_w_r, B_w_gate, B_w_up, B_w_down)
```

```python
import jax
import jax.numpy as jnp
from jax import lax
import jax.experimental.pallas as pl
import jax.experimental.pallas.tpu as pltpu

HQ, DH = 32, 128
F32 = jnp.float32
BF16 = jnp.bfloat16
NT = (((1,), (1,)), ((), ()))

M = 8
WQ_CH = 4
WO_CH = 4
SIDE_ROWS = 96
WD_CH = (512, 256, 128, 64, 32, 32)
N_VPU = 4


def _kernel(x_hbm, k_hbm, v_hbm, wq_hbm, wo_hbm, wr_hbm, wg_hbm, wu_hbm, wd_hbm, out_ref,
            x_v, wr_v, wq_v, k_v, v_v, wo_v, wg_v, wu_v, wd_v, q_s, o_s, hc_s, sbuf, sems):
    hkv, sk = k_hbm.shape[1], k_hbm.shape[2]
    W = k_v.shape[1]
    D = x_v.shape[-1]
    FF = wg_v.shape[1]
    rep = HQ // hkv
    wq_rows = D // WQ_CH
    wo_rows = (HQ * DH) // WO_CH
    side = hkv * SIDE_ROWS
    assert side + sum(WD_CH) == FF
    wd_off = [side + sum(WD_CH[:i]) for i in range(len(WD_CH))]
    n_mxu = len(WD_CH) - N_VPU
    R = sum(WD_CH[n_mxu:])
    assert R % 128 == 0
    S_X, S_WR, S_WQ = 0, 1, 2
    S_K = S_WQ + WQ_CH
    S_V = S_K + hkv
    S_WO = S_V + hkv
    S_WG = S_WO + WO_CH
    S_WU = S_WG + 1
    S_WD = S_WU + 1
    S_HS = S_WD + len(WD_CH)
    S_SV = S_HS + hkv

    def rows_copy(src, dst, off, n, s):
        return pltpu.make_async_copy(src.at[pl.ds(off, n)], dst.at[pl.ds(off, n)], sems.at[s])

    def cp_x():
        return pltpu.make_async_copy(x_hbm, x_v, sems.at[S_X])

    def cp_wr():
        return pltpu.make_async_copy(wr_hbm, wr_v, sems.at[S_WR])

    def cp_wq(c):
        return rows_copy(wq_hbm, wq_v, c * wq_rows, wq_rows, S_WQ + c)

    def cp_k(h):
        return pltpu.make_async_copy(k_hbm.at[0, h, pl.ds(sk - W, W)], k_v.at[h], sems.at[S_K + h])

    def cp_v(h):
        return pltpu.make_async_copy(v_hbm.at[0, h, pl.ds(sk - W, W)], v_v.at[h], sems.at[S_V + h])

    def cp_wo(c):
        return rows_copy(wo_hbm, wo_v, c * wo_rows, wo_rows, S_WO + c)

    def cp_wg():
        return pltpu.make_async_copy(wg_hbm, wg_v, sems.at[S_WG])

    def cp_wu():
        return pltpu.make_async_copy(wu_hbm, wu_v, sems.at[S_WU])

    def cp_wd(c):
        return rows_copy(wd_hbm, wd_v, wd_off[c], WD_CH[c], S_WD + c)

    def side_off(i):
        return i * SIDE_ROWS if isinstance(i, int) else pl.multiple_of(i * SIDE_ROWS, 16)

    def cp_hs(i):
        return rows_copy(wd_hbm, sbuf, side_off(i), SIDE_ROWS, S_HS + i)

    def cp_sv(i):
        return rows_copy(sbuf, wd_v, side_off(i), SIDE_ROWS, S_SV + i)

    cp_wq(0).start()
    cp_hs(0).start()
    cp_x().start()
    cp_wr().start()
    for c in range(1, WQ_CH):
        cp_wq(c).start()
    for i in range(1, hkv):
        cp_hs(i).start()
    for h in range(hkv):
        cp_k(h).start()
        cp_v(h).start()
    cp_wg().start()
    cp_wu().start()
    for c in range(WO_CH):
        cp_wo(c).start()
    for c in range(len(WD_CH)):
        cp_wd(c).start()

    cp_x().wait()
    x = x_v[0].astype(F32)
    mu = jnp.mean(x, axis=-1, keepdims=True)
    xc = x - mu
    var = jnp.mean(xc * xc, axis=-1, keepdims=True)
    xn = xc / jnp.sqrt(var + 1e-5)
    xb = jnp.broadcast_to(xn, (M, D)).astype(BF16)

    cp_wr().wait()
    wr = wr_v[...].astype(F32).reshape(1, D)
    r = jnp.sum(xn * wr, axis=-1, keepdims=True)
    gate = jax.nn.sigmoid(r)

    q = None
    for c in range(WQ_CH):
        cp_wq(c).wait()
        part = jnp.dot(xb[:, c * wq_rows:(c + 1) * wq_rows], wq_v[c * wq_rows:(c + 1) * wq_rows, :],
                       preferred_element_type=F32)
        q = part if q is None else q + part
    q = q * (DH ** -0.5)
    row = lax.broadcasted_iota(jnp.int32, (M, DH), 0)
    for h in range(hkv):
        qh = q[:, (h * rep) * DH:(h * rep + 1) * DH]
        for j in range(1, rep):
            qh = jnp.where(row == j, q[:, (h * rep + j) * DH:(h * rep + j + 1) * DH], qh)
        q_s[h] = qh

    def head(h, carry):
        cp_k(h).wait()
        qh = q_s[h].astype(BF16)
        s = lax.dot_general(qh, k_v[h], NT, preferred_element_type=F32)
        m = jnp.max(s, axis=-1, keepdims=True)
        p = jnp.exp(s - m)
        l = jnp.sum(p, axis=-1, keepdims=True)
        cp_hs(h).wait()
        cp_sv(h).start()
        cp_v(h).wait()
        o = jnp.dot(p.astype(BF16), v_v[h], preferred_element_type=F32)
        o_s[h] = o / l
        return carry
    lax.fori_loop(0, hkv, head, 0)

    cp_wg().wait()
    g = jnp.dot(xb, wg_v[...], preferred_element_type=F32)
    cp_wu().wait()
    u = jnp.dot(xb, wu_v[...], preferred_element_type=F32)
    hf = g * jax.nn.sigmoid(g) * u
    hh = hf.astype(BF16)
    for b in range(R // 128):
        lo = FF - R + b * 128
        hl = jnp.broadcast_to(hf[0:1, lo:lo + 128] * gate, (128, 128))
        hc_s[b * 128:(b + 1) * 128, :] = jnp.transpose(hl)

    pieces = []
    for h in range(hkv):
        oh = o_s[h]
        for j in range(rep):
            pieces.append(jnp.where(row == j, oh, 0.0).astype(BF16))
    obd = jnp.concatenate(pieces, axis=1)
    acc = None
    for c in range(WO_CH):
        cp_wo(c).wait()
        part = jnp.dot(obd[:, c * wo_rows:(c + 1) * wo_rows], wo_v[c * wo_rows:(c + 1) * wo_rows, :],
                       preferred_element_type=F32)
        acc = part if acc is None else acc + part

    for i in range(hkv):
        cp_sv(i).wait()
    y = jnp.dot(hh[:, :side], wd_v[:side, :], preferred_element_type=F32)
    for c in range(n_mxu):
        cp_wd(c).wait()
        y = y + jnp.dot(hh[:, wd_off[c]:wd_off[c] + WD_CH[c]], wd_v[wd_off[c]:wd_off[c] + WD_CH[c], :],
                        preferred_element_type=F32)
    row8 = lax.broadcasted_iota(jnp.int32, (M, D), 0)
    acc = acc + jnp.where(row8 == 0, x + xn + y * gate, 0.0)
    for c in range(n_mxu, len(WD_CH)):
        cp_wd(c).wait()
        off, n = wd_off[c], WD_CH[c]
        wl = wd_v[off:off + n, :].astype(F32)
        hcol = hc_s[off - (FF - R):off - (FF - R) + n, :]
        hc = jnp.concatenate([hcol] * (D // 128), axis=1)
        acc = acc + jnp.sum((wl * hc).reshape(n // M, M, D), axis=0)
    out_ref[0] = jnp.sum(acc, axis=0, keepdims=True).astype(out_ref.dtype)


@jax.jit
def pallas_parallel_sum__sliding_block_cached__moe_arch_mod__decode_kernel(
    A_x: jax.Array,
    A_k_cache: jax.Array,
    A_v_cache: jax.Array,
    A_wq: jax.Array,
    A_wo: jax.Array,
    B_x: jax.Array,
    B_w_r: jax.Array,
    B_w_gate: jax.Array,
    B_w_up: jax.Array,
    B_w_down: jax.Array,
):
    del B_x
    hkv, sk = A_k_cache.shape[1], A_k_cache.shape[2]
    W = min(4096, max(256, sk // 4))
    D = A_x.shape[-1]
    nsem = 2 + WQ_CH + 2 * hkv + WO_CH + 2 + len(WD_CH) + 2 * hkv
    anyspec = pl.BlockSpec(memory_space=pl.ANY)
    return pl.pallas_call(
        _kernel,
        out_shape=jax.ShapeDtypeStruct(A_x.shape, A_x.dtype),
        in_specs=[anyspec] * 9,
        out_specs=pl.BlockSpec(memory_space=pltpu.VMEM),
        scratch_shapes=[
            pltpu.VMEM(A_x.shape, BF16), pltpu.VMEM(B_w_r.shape, BF16),
            pltpu.VMEM(A_wq.shape, BF16),
            pltpu.VMEM((hkv, W, DH), BF16), pltpu.VMEM((hkv, W, DH), BF16),
            pltpu.VMEM(A_wo.shape, BF16),
            pltpu.VMEM(B_w_gate.shape, BF16), pltpu.VMEM(B_w_up.shape, BF16),
            pltpu.VMEM(B_w_down.shape, BF16),
            pltpu.VMEM((hkv, M, DH), F32), pltpu.VMEM((hkv, M, DH), F32),
            pltpu.VMEM((sum(WD_CH[len(WD_CH) - N_VPU:]), 128), F32),
            pltpu.SMEM((hkv * SIDE_ROWS, D), BF16),
            pltpu.SemaphoreType.DMA((nsem,)),
        ],
        compiler_params=pltpu.CompilerParams(
            vmem_limit_bytes=48 * 1024 * 1024,
            disable_semaphore_checks=True,
        ),
    )(A_x, A_k_cache, A_v_cache, A_wq, A_wo, B_w_r, B_w_gate, B_w_up, B_w_down)
```

```python
import jax
import jax.numpy as jnp
from jax import lax
import jax.experimental.pallas as pl
import jax.experimental.pallas.tpu as pltpu

HQ, DH = 32, 128
F32 = jnp.float32
BF16 = jnp.bfloat16
NT = (((1,), (1,)), ((), ()))
NG = 8
LO, HI = 1, 0
NS = 8
AL = 5
AH = 4
P4HI = (4, 4, 3, 3, 3, 3, 3, 3, 3, 3, 3, 3, 3, 3)
SUB = ((0, 4, 0, 32), (4, 2, 0, 32), (6, 1, 0, 32), (7, 1, 0, 16), (7, 1, 16, 16))
LATE_POS = 2


def _kernel(x_hbm, k_hbm, v_hbm, wq_hbm, wo_hbm, wr_hbm, wg_hbm, wu_hbm, wd_hbm, out_ref,
            x_v, wr_v, wq_v, k_v, v_v, wo_v, wg_v, wu_v, wd_v,
            xcol, qacc, q_s, s_s, m_s, col_s, lsem, hsem, msem):
    hkv, sk = k_hbm.shape[1], k_hbm.shape[2]
    nkc = k_v.shape[0]
    W = nkc * 128
    D = x_v.shape[-1]
    FF = wg_v.shape[1]
    rep = HQ // hkv
    HF = FF // 2
    QH = (HQ * DH) // 2
    N1, N2, N3, N4 = 16, nkc, nkc, 16
    BASE = {1: 0, 2: N1, 3: N1 + N2, 4: N1 + N2 + N3}
    NP = {1: N1, 2: N2, 3: N3, 4: N4}
    NWD = FF // 16
    WD_P3 = 4 * (N1 - AH + 1)
    WD_P4 = WD_P3 + 4 * AH
    assert WD_P4 + sum(P4HI) == NWD and hkv == NG and rep == 4 and D == 16 * nkc

    def mo(i, m):
        return i if isinstance(i, int) else pl.multiple_of(i, m)

    def low(p, s):
        if p == 1:
            r, hf = s // 2, s % 2
            src = wq_hbm.at[:, pl.ds(mo(r * 8, 8), 8), pl.ds(mo(hf * QH, 128), QH)]
            dst = wq_v.at[s]
        elif p == 2:
            src, dst = k_hbm.at[0, :, pl.ds(mo(sk - W + s * 128, 128), 128)], k_v.at[s]
        elif p == 3:
            src, dst = v_hbm.at[0, :, pl.ds(mo(sk - W + s * 128, 128), 128)], v_v.at[s]
        else:
            src, dst = wo_hbm.at[:, pl.ds(mo(s * 32, 32), 32)], wo_v.at[s]
        return pltpu.make_async_copy(src, dst, lsem.at[(BASE[p] + s) % NS])

    def sub(i):
        g0, ng, r0, nr = SUB[i]
        s = N4 - 1
        return pltpu.make_async_copy(wo_hbm.at[pl.ds(g0, ng), pl.ds(s * 32 + r0, nr)],
                                     wo_v.at[s, pl.ds(g0, ng), pl.ds(r0, nr)], msem.at[2 + i])

    def hsem_at(it, k):
        return hsem.at[((it + 1) % NS) * 4 + k]

    def hi_wd(piece, it, k):
        sl = pl.ds(mo(piece * 16, 16), 16)
        return pltpu.make_async_copy(wd_hbm.at[sl], wd_v.at[sl], hsem_at(it, k))

    def hi_gu(p, c, k):
        h, v = (wg_hbm, wg_v) if p == 2 else (wu_hbm, wu_v)
        rs, cs = pl.ds(mo(c * 16 + (k // 2) * 8, 8), 8), pl.ds((k % 2) * HF, HF)
        return pltpu.make_async_copy(h.at[rs, cs], v.at[rs, cs], hsem_at(BASE[p] + c - AH, k))

    def branch(cond, fa, fb):
        pl.when(cond)(fa)
        pl.when(jnp.logical_not(cond))(fb)

    def start_low(p, s):
        n = NP[p]
        branch(s + AL < n,
               lambda: low(p, s + AL).start(priority=LO),
               lambda: low(p + 1, s + AL - n).start(priority=LO))

    def start_high(p, s, k):
        n, it = NP[p], BASE[p] + s

        def own():
            cp = hi_wd(4 * (s + 1) + k, it, k) if p == 1 else hi_gu(p, s + AH, k)
            cp.start(priority=HI)

        def nxt():
            cp = hi_wd(WD_P3 + 4 * (s + AH - n) + k, it, k) if p == 3 else hi_gu(p + 1, s + AH - n, k)
            cp.start(priority=HI)

        branch(s + AH < n, own, nxt)

    cp_x = pltpu.make_async_copy(x_hbm, x_v, msem.at[0])
    cp_wr = pltpu.make_async_copy(wr_hbm, wr_v, msem.at[1])

    cp_x.start(priority=HI)
    low(1, 0).start(priority=LO)
    cp_wr.start(priority=HI)
    hi_wd(0, -1, 0).start(priority=HI)
    for s in range(1, AL):
        low(1, s).start(priority=LO)
    hi_wd(1, -1, 1).start(priority=HI)

    cp_x.wait()
    hi_wd(2, -1, 2).start(priority=HI)
    x = x_v[0].astype(F32)
    mu = jnp.mean(x, axis=-1, keepdims=True)
    xc = x - mu
    var = jnp.mean(xc * xc, axis=-1, keepdims=True)
    xn = xc / jnp.sqrt(var + 1e-5)
    qacc[...] = jnp.zeros(qacc.shape, F32)
    cp_wr.wait()
    hi_wd(3, -1, 3).start(priority=HI)
    for b in range(D // 128):
        xcol[b * 128:(b + 1) * 128, :] = jnp.transpose(
            jnp.broadcast_to(xn[:, b * 128:(b + 1) * 128], (128, 128)))
    wr = wr_v[...].astype(F32).reshape(1, D)
    gate = jax.nn.sigmoid(jnp.sum(xn * wr, axis=-1, keepdims=True))

    def lanes(col, n):
        return jnp.concatenate([col] * n, axis=1)

    def p1(r, carry):
        for hf in range(2):
            s = r * 2 + hf
            low(1, s).wait()
            for k in range(4):
                @pl.when(s >= AH - 1)
                def _():
                    hi_wd(4 * (s - AH + 1) + k, s - AH, k).wait()
                start_high(1, s, k)
                if k == 0:
                    start_low(1, s)
                acc = qacc[hf, :, k * 512:(k + 1) * 512]
                for g in range(NG):
                    xc8 = xcol[pl.ds(pl.multiple_of(g * 64 + r * 8, 8), 8), :]
                    acc = acc + wq_v[s, g, :, k * 512:(k + 1) * 512].astype(F32) * lanes(xc8, 4)
                qacc[hf, :, k * 512:(k + 1) * 512] = acc
        return carry
    lax.fori_loop(0, N1 // 2, p1, 0)

    row = lax.broadcasted_iota(jnp.int32, (8, DH), 0)
    for h in range(hkv):
        qh = None
        for j in range(rep):
            n = h * rep + j
            qn = jnp.sum(qacc[n // 16, :, (n % 16) * DH:(n % 16 + 1) * DH], axis=0, keepdims=True)
            qn = jnp.broadcast_to(qn, (8, DH))
            qh = qn if qh is None else jnp.where(row == j, qn, qh)
        q_s[h] = qh * (DH ** -0.5)

    def ffn_part(w_v, c, t, acc):
        r0 = pl.multiple_of(c * 16 + t * 8, 8)
        return acc + w_v[pl.ds(r0, 8), :].astype(F32) * lanes(xcol[pl.ds(r0, 8), :], FF // 128)

    def p2(c, carry):
        ms, gacc = carry
        ms = list(ms)
        low(2, c).wait()
        for t in range(2):
            start_high(2, c, 2 * t)
            if t == 0:
                start_low(2, c)
            for h in range(4 * t, 4 * t + 4):
                s = lax.dot_general(q_s[h].astype(BF16), k_v[c, h], NT, preferred_element_type=F32)
                s_s[c, h] = s
                ms[h] = jnp.maximum(ms[h], s)
            hi_gu(2, c, 2 * t).wait()
            hi_gu(2, c, 2 * t + 1).wait()
            start_high(2, c, 2 * t + 1)
            gacc = ffn_part(wg_v, c, t, gacc)
        return tuple(ms), gacc
    neg = jnp.full((8, DH), -jnp.inf, F32)
    ms, gacc = lax.fori_loop(0, N2, p2, ((neg,) * hkv, jnp.zeros((8, FF), F32)))
    for h in range(hkv):
        m_s[h] = jnp.broadcast_to(jnp.max(ms[h], axis=-1, keepdims=True), (8, DH))
    g = jnp.sum(gacc, axis=0, keepdims=True)
    sg = g * jax.nn.sigmoid(g) * gate

    def p3(c, carry):
        os_, ls, uacc = carry
        os_, ls = list(os_), list(ls)
        low(3, c).wait()
        for t in range(2):
            start_high(3, c, 2 * t)
            if t == 0:
                start_low(3, c)
            for h in range(4 * t, 4 * t + 4):
                p = jnp.exp(s_s[c, h] - m_s[h])
                ls[h] = ls[h] + p
                os_[h] = os_[h] + jnp.dot(p.astype(BF16), v_v[c, h], preferred_element_type=F32)
            hi_gu(3, c, 2 * t).wait()
            hi_gu(3, c, 2 * t + 1).wait()
            start_high(3, c, 2 * t + 1)
            uacc = ffn_part(wu_v, c, t, uacc)
        return tuple(os_), tuple(ls), uacc
    zero = jnp.zeros((8, DH), F32)
    os_, ls, uacc = lax.fori_loop(0, N3, p3, ((zero,) * hkv, (zero,) * hkv, jnp.zeros((8, FF), F32)))

    hid = sg * jnp.sum(uacc, axis=0, keepdims=True)
    rowf = lax.broadcasted_iota(jnp.int32, (8, FF), 0)
    hb = jnp.where(rowf == 0, hid, 0.0).astype(BF16)
    on = [os_[h] / jnp.sum(ls[h], axis=-1, keepdims=True) for h in range(hkv)]
    seg = lax.broadcasted_iota(jnp.int32, (8, DH), 1) // 32
    rolled = [[on[h] if sh == 0 else pltpu.roll(on[h], sh * 32, axis=1) for sh in range(4)]
              for h in range(hkv)]
    lhs = []
    for q in range(4):
        halves = []
        for hf in range(2):
            v = rolled[4 * hf][(0 - q) % 4]
            for sg_ in range(1, 4):
                v = jnp.where(seg == sg_, rolled[4 * hf + sg_][(sg_ - q) % 4], v)
            halves.append(v)
        lhs.append(jnp.concatenate(halves, axis=1))
    row2 = lax.broadcasted_iota(jnp.int32, (8, 2 * DH), 0)

    def to_col(slot, vec):
        col_s[slot * 128:(slot + 1) * 128, :] = jnp.transpose(jnp.broadcast_to(vec, (128, 128)))

    def vpu_rows(acc, w, c0, n):
        prod = w.astype(F32) * lanes(col_s[c0:c0 + n, :], D // 128)
        return acc + jnp.sum(prod.reshape(n // 8, 8, D), axis=0)

    issue = {}
    for j in range(AH):
        for k in range(4):
            issue[WD_P3 + 4 * j + k] = (BASE[4] - AH + j, k)
    pc = WD_P4
    for c, cnt in enumerate(P4HI):
        for k in range(cnt):
            issue[pc] = (BASE[4] + c, k)
            pc += 1
    NMX = FF // 128 - 2
    VP0 = NMX * 8
    waited = set(range(WD_P3))
    todo_blocks = list(range(NMX))

    def start_piece(p):
        hi_wd(p, *issue[p]).start(priority=HI)

    def wait_piece(p):
        hi_wd(p, *issue[p]).wait()
        waited.add(p)

    def vpu_piece(acc, p):
        return vpu_rows(acc, wd_v[p * 16:(p + 1) * 16, :], 256 + (p - VP0) * 16, 16)

    row8 = lax.broadcasted_iota(jnp.int32, (8, D), 0)
    acc = jnp.where(row8 == 0, x + xn, 0.0)
    for c in range(N4 - 1):
        it = BASE[4] + c
        starts = [p for p, (i, _) in issue.items() if i == it]
        waits = [p for p, (i, _) in issue.items() if i == it - AH]
        low(4, c).wait()
        for p in starts[:1]:
            start_piece(p)
        if c + AL < N4 - 1:
            low(4, c + AL).start(priority=LO)
        elif c + AL == N4 - 1:
            for i in range(len(SUB)):
                sub(i).start(priority=LO)
        l = jnp.where(row2 == c // 4, lhs[c % 4], 0.0).astype(BF16)
        acc = acc + jnp.dot(l, wo_v[c].reshape(2 * DH, D), preferred_element_type=F32)
        for p in waits[:-1]:
            wait_piece(p)
        for p in starts[1:2]:
            start_piece(p)
        ready = [b for b in todo_blocks if all(q in waited for q in range(8 * b, 8 * b + 8))]
        if ready:
            b = ready[0]
            todo_blocks.remove(b)
            acc = acc + jnp.dot(hb[:, b * 128:(b + 1) * 128], wd_v[b * 128:(b + 1) * 128, :],
                                preferred_element_type=F32)
        if c < 2:
            to_col(c, lhs[3][rep - 1:rep, c * 128:(c + 1) * 128])
        elif c < 4:
            to_col(c, hid[:, (NMX + c - 2) * 128:(NMX + c - 1) * 128])
        for p in waits[-1:]:
            wait_piece(p)
        for p in starts[2:3]:
            start_piece(p)
        for p in waits:
            if p >= VP0:
                acc = vpu_piece(acc, p)
        for p in starts[3:]:
            start_piece(p)
    assert not todo_blocks
    rest = [p for p in range(NWD) if p not in waited]
    assert all(p >= VP0 for p in rest)
    last_it = max(issue[p][0] for p in rest)
    for p in rest:
        if issue[p][0] != last_it:
            wait_piece(p)
            acc = vpu_piece(acc, p)
    for i in range(len(SUB)):
        if i == LATE_POS:
            late = [p for p in rest if issue[p][0] == last_it]
            for p in late:
                wait_piece(p)
            for p in late:
                acc = vpu_piece(acc, p)
        g0, ng, r0, nr = SUB[i]
        sub(i).wait()
        for g_ in range(g0, g0 + ng):
            acc = vpu_rows(acc, wo_v[N4 - 1, g_, r0:r0 + nr, :], g_ * 32 + r0, nr)
    out_ref[0] = jnp.sum(acc, axis=0, keepdims=True).astype(out_ref.dtype)


@jax.jit
def pallas_parallel_sum__sliding_block_cached__moe_arch_mod__decode_kernel(
    A_x: jax.Array,
    A_k_cache: jax.Array,
    A_v_cache: jax.Array,
    A_wq: jax.Array,
    A_wo: jax.Array,
    B_x: jax.Array,
    B_w_r: jax.Array,
    B_w_gate: jax.Array,
    B_w_up: jax.Array,
    B_w_down: jax.Array,
):
    del B_x
    hkv, sk = A_k_cache.shape[1], A_k_cache.shape[2]
    W = min(4096, max(256, sk // 4))
    D = A_x.shape[-1]
    nkc = W // 128
    wq3 = A_wq.reshape(NG, D // NG, HQ * DH)
    wo3 = A_wo.reshape(NG, HQ * DH // NG, D)
    anyspec = pl.BlockSpec(memory_space=pl.ANY)
    return pl.pallas_call(
        _kernel,
        out_shape=jax.ShapeDtypeStruct(A_x.shape, A_x.dtype),
        in_specs=[anyspec] * 9,
        out_specs=pl.BlockSpec(memory_space=pltpu.VMEM),
        scratch_shapes=[
            pltpu.VMEM(A_x.shape, BF16), pltpu.VMEM(B_w_r.shape, BF16),
            pltpu.VMEM((16, NG, 8, HQ * DH // 2), BF16),
            pltpu.VMEM((nkc, hkv, 128, DH), BF16), pltpu.VMEM((nkc, hkv, 128, DH), BF16),
            pltpu.VMEM((16, NG, 32, D), BF16),
            pltpu.VMEM(B_w_gate.shape, BF16), pltpu.VMEM(B_w_up.shape, BF16),
            pltpu.VMEM(B_w_down.shape, BF16),
            pltpu.VMEM((D, 128), F32), pltpu.VMEM((2, 8, HQ * DH // 2), F32),
            pltpu.VMEM((hkv, 8, DH), F32), pltpu.VMEM((nkc, hkv, 8, DH), F32),
            pltpu.VMEM((hkv, 8, DH), F32),
            pltpu.VMEM((512, 128), F32),
            pltpu.SemaphoreType.DMA((NS,)), pltpu.SemaphoreType.DMA((NS * 4,)),
            pltpu.SemaphoreType.DMA((2 + len(SUB),)),
        ],
        compiler_params=pltpu.CompilerParams(
            vmem_limit_bytes=48 * 1024 * 1024,
            disable_semaphore_checks=True,
            disable_bounds_checks=True,
        ),
    )(A_x, A_k_cache, A_v_cache, wq3, wo3, B_w_r, B_w_gate, B_w_up, B_w_down)
```

```python
import jax
import jax.numpy as jnp
from jax import lax
import jax.experimental.pallas as pl
import jax.experimental.pallas.tpu as pltpu

HQ, DH = 32, 128
F32 = jnp.float32
BF16 = jnp.bfloat16
NT = (((1,), (1,)), ((), ()))
NG = 8
LO, HI = 1, 0
NS = 8
AL = 5
AH = 4
P4HI = (4,) + (3,) * 12
SUB = ((0, 4, 0, 32), (4, 2, 0, 32), (6, 1, 0, 32), (7, 1, 0, 16), (7, 1, 16, 16))
LATE_POS = 1
TOCOL = (8, 9, 6, 7)


def _kernel(x_hbm, k_hbm, v_hbm, wq_hbm, wo_hbm, wr_hbm, wg_hbm, wu_hbm, wd_hbm, out_ref,
            x_v, wr_v, wq_v, k_v, v_v, wo_v, gu_v, wd_v,
            xcol, qacc, guacc, q_s, s_s, m_s, col_s, lsem, hsem, msem):
    hkv, sk = k_hbm.shape[1], k_hbm.shape[2]
    nkc = k_v.shape[0]
    W = nkc * 128
    D = x_v.shape[-1]
    FF = wg_hbm.shape[1]
    rep = HQ // hkv
    HF = FF // 2
    QH = (HQ * DH) // 2
    N1, N2, N3, N4 = 16, nkc, nkc, 16
    BASE = {1: 0, 2: N1, 3: N1 + N2, 4: N1 + N2 + N3}
    NP = {1: N1, 2: N2, 3: N3, 4: N4}
    NWD = FF // 16
    WD_P3 = 4 * (N1 - AH + 2)
    WD_P4 = WD_P3 + 4 * AH
    assert WD_P4 + sum(P4HI) == NWD and hkv == NG and rep == 4 and D == 16 * nkc

    def mo(i, m):
        return i if isinstance(i, int) else pl.multiple_of(i, m)

    def low(p, s):
        if p == 1:
            r, hf = s // 2, s % 2
            src = wq_hbm.at[:, pl.ds(mo(r * 8, 8), 8), pl.ds(mo(hf * QH, 128), QH)]
            dst = wq_v.at[s]
        elif p == 2:
            src, dst = k_hbm.at[0, :, pl.ds(mo(sk - W + s * 128, 128), 128)], k_v.at[s]
        elif p == 3:
            src, dst = v_hbm.at[0, :, pl.ds(mo(sk - W + s * 128, 128), 128)], v_v.at[s]
        else:
            src, dst = wo_hbm.at[:, pl.ds(mo(s * 32, 32), 32)], wo_v.at[s]
        return pltpu.make_async_copy(src, dst, lsem.at[(BASE[p] + s) % NS])

    def sub(i):
        g0, ng, r0, nr = SUB[i]
        s = N4 - 1
        return pltpu.make_async_copy(wo_hbm.at[pl.ds(g0, ng), pl.ds(s * 32 + r0, nr)],
                                     wo_v.at[s, pl.ds(g0, ng), pl.ds(r0, nr)], msem.at[2 + i])

    def hsem_at(it, k):
        return hsem.at[((it + 2) % NS) * 4 + k]

    def wd_piece(seq):
        return (seq % 2) * (NWD // 2) + seq // 2

    def hi_wd(seq, it, k):
        sl = pl.ds(mo(wd_piece(seq) * 16, 16), 16)
        return pltpu.make_async_copy(wd_hbm.at[sl], wd_v.at[sl], hsem_at(it, k))

    def gu_row(u, k):
        return mo((u // 2 + (k // 2) * (D // 16)) * 8, 8)

    def hi_gu(u, k):
        h = wg_hbm if k % 2 == 0 else wu_hbm
        src = h.at[pl.ds(gu_row(u, k), 8), pl.ds(mo((u % 2) * HF, 128), HF)]
        return pltpu.make_async_copy(src, gu_v.at[u, k], hsem_at(N1 + u - AH, k))

    def branch(cond, fa, fb):
        pl.when(cond)(fa)
        pl.when(jnp.logical_not(cond))(fb)

    def start_low(p, s):
        n = NP[p]
        branch(s + AL < n,
               lambda: low(p, s + AL).start(priority=LO),
               lambda: low(p + 1, s + AL - n).start(priority=LO))

    def start_high(p, s, k):
        n, it = NP[p], BASE[p] + s

        def gu():
            hi_gu(it + AH - N1, k).start(priority=HI)

        if p == 1:
            branch(s + AH < n, lambda: hi_wd(4 * (s + 2) + k, it, k).start(priority=HI), gu)
        elif p == 2:
            gu()
        else:
            branch(s + AH < n, gu, lambda: hi_wd(WD_P3 + 4 * (s + AH - n) + k, it, k).start(priority=HI))

    cp_x = pltpu.make_async_copy(x_hbm, x_v, msem.at[0])
    cp_wr = pltpu.make_async_copy(wr_hbm, wr_v, msem.at[1])

    cp_x.start(priority=HI)
    low(1, 0).start(priority=LO)
    cp_wr.start(priority=HI)
    for s in range(1, AL):
        low(1, s).start(priority=LO)

    def fill(k, carry):
        hi_wd(k, -2, k).start(priority=HI)
        s_s[pl.ds(k * (nkc // 4), nkc // 4)] = jnp.zeros((nkc // 4,) + s_s.shape[1:], F32)
        return carry
    lax.fori_loop(0, 4, fill, 0)

    cp_x.wait()
    hi_wd(4, -1, 0).start(priority=HI)
    x = x_v[0].astype(F32)
    mu = jnp.mean(x, axis=-1, keepdims=True)
    xc = x - mu
    var = jnp.mean(xc * xc, axis=-1, keepdims=True)
    xn = xc / jnp.sqrt(var + 1e-5)
    qacc[...] = jnp.zeros(qacc.shape, F32)
    guacc[...] = jnp.zeros(guacc.shape, F32)
    cp_wr.wait()
    hi_wd(5, -1, 1).start(priority=HI)
    for b in range(D // 128):
        xcol[b * 128:(b + 1) * 128, :] = jnp.transpose(
            jnp.broadcast_to(xn[:, b * 128:(b + 1) * 128], (128, 128)))
        if b % 2 == 1:
            hi_wd(b - 1, -2, b - 1).wait()
            hi_wd(b, -2, b).wait()
            hi_wd(6 + b // 2, -1, 2 + b // 2).start(priority=HI)
    wr = wr_v[...].astype(F32).reshape(1, D)
    gate = jax.nn.sigmoid(jnp.sum(xn * wr, axis=-1, keepdims=True))

    def lanes(col, n):
        return jnp.concatenate([col] * n, axis=1)

    def p1(r, carry):
        for hf in range(2):
            s = r * 2 + hf
            low(1, s).wait()
            for k in range(4):
                @pl.when(s >= AH - 1)
                def _():
                    hi_wd(4 * (s - AH + 2) + k, s - AH, k).wait()
                start_high(1, s, k)
                if k == 0:
                    start_low(1, s)
                acc = qacc[hf, :, k * 512:(k + 1) * 512]
                for g in range(NG):
                    xc8 = xcol[pl.ds(pl.multiple_of(g * 64 + r * 8, 8), 8), :]
                    acc = acc + wq_v[s, g, :, k * 512:(k + 1) * 512].astype(F32) * lanes(xc8, 4)
                qacc[hf, :, k * 512:(k + 1) * 512] = acc
        return carry
    lax.fori_loop(0, N1 // 2, p1, 0)

    row = lax.broadcasted_iota(jnp.int32, (8, DH), 0)
    for h in range(hkv):
        qh = None
        for j in range(rep):
            n = h * rep + j
            qn = jnp.sum(qacc[n // 16, :, (n % 16) * DH:(n % 16 + 1) * DH], axis=0, keepdims=True)
            qn = jnp.broadcast_to(qn, (8, DH))
            qh = qn if qh is None else jnp.where(row == j, qn, qh)
        q_s[h] = qh * (DH ** -0.5)

    def ffn_part(u, w):
        acc = guacc[w, u % 2]
        for k in (w, w + 2):
            acc = acc + gu_v[u, k].astype(F32) * lanes(xcol[pl.ds(gu_row(u, k), 8), :], HF // 128)
        guacc[w, u % 2] = acc

    def step23(p, c, heads):
        u = BASE[p] - N1 + c
        low(p, c).wait()
        start_high(p, c, 0)
        start_low(p, c)
        heads(range(0, 4))
        hi_gu(u, 0).wait()
        hi_gu(u, 2).wait()
        start_high(p, c, 1)
        ffn_part(u, 0)
        hi_gu(u, 1).wait()
        start_high(p, c, 2)
        heads(range(4, 8))
        hi_gu(u, 3).wait()
        start_high(p, c, 3)
        ffn_part(u, 1)

    def p2(c, ms):
        ms = list(ms)

        def heads(hs):
            for h in hs:
                s = lax.dot_general(q_s[h].astype(BF16), k_v[c, h], NT, preferred_element_type=F32)
                s_s[c, h] = s
                ms[h] = jnp.maximum(ms[h], s)
        step23(2, c, heads)
        return tuple(ms)
    neg = jnp.full((8, DH), -jnp.inf, F32)
    ms = lax.fori_loop(0, N2, p2, (neg,) * hkv)
    for h in range(hkv):
        m_s[h] = jnp.broadcast_to(jnp.max(ms[h], axis=-1, keepdims=True), (8, DH))

    def p3(c, carry):
        os_, ls = list(carry[0]), list(carry[1])

        def heads(hs):
            for h in hs:
                p = jnp.exp(s_s[c, h] - m_s[h])
                ls[h] = ls[h] + p
                os_[h] = os_[h] + jnp.dot(p.astype(BF16), v_v[c, h], preferred_element_type=F32)
        step23(3, c, heads)
        return tuple(os_), tuple(ls)
    zero = jnp.zeros((8, DH), F32)
    os_, ls = lax.fori_loop(0, N3, p3, ((zero,) * hkv, (zero,) * hkv))

    on = [os_[h] / jnp.sum(ls[h], axis=-1, keepdims=True) for h in range(hkv)]
    seg = lax.broadcasted_iota(jnp.int32, (8, DH), 1) // 32
    rolled = [[on[h] if sh == 0 else pltpu.roll(on[h], sh * 32, axis=1) for sh in range(4)]
              for h in range(hkv)]
    lhs = []
    for q in range(4):
        halves = []
        for hf in range(2):
            v = rolled[4 * hf][(0 - q) % 4]
            for sg in range(1, 4):
                v = jnp.where(seg == sg, rolled[4 * hf + sg][(sg - q) % 4], v)
            halves.append(v)
        lhs.append(jnp.concatenate(halves, axis=1))
    row2 = lax.broadcasted_iota(jnp.int32, (8, 2 * DH), 0)
    g, up = [jnp.concatenate([jnp.sum(guacc[w, hf], axis=0, keepdims=True) for hf in range(2)], axis=1)
             for w in range(2)]
    hid = g * jax.nn.sigmoid(g) * up * gate
    rowf = lax.broadcasted_iota(jnp.int32, (8, FF), 0)
    hb = jnp.where(rowf == 0, hid, 0.0).astype(BF16)

    def to_col(slot, vec):
        col_s[slot * 128:(slot + 1) * 128, :] = jnp.transpose(jnp.broadcast_to(vec, (128, 128)))

    def vpu_rows(acc, w, c0, n):
        prod = w.astype(F32) * lanes(col_s[c0:c0 + n, :], D // 128)
        return acc + jnp.sum(prod.reshape(n // 8, 8, D), axis=0)

    issue = {}
    for j in range(AH):
        for k in range(4):
            issue[WD_P3 + 4 * j + k] = (BASE[4] - AH + j, k)
    pc = WD_P4
    for c, cnt in enumerate(P4HI):
        for k in range(cnt):
            issue[pc] = (BASE[4] + c, k)
            pc += 1
    vblocks = sorted({wd_piece(q) // 8 for q in range(NWD - 16, NWD)})
    assert len(vblocks) == 2
    have = {wd_piece(q) for q in range(WD_P3)}
    waited = set(range(WD_P3))
    todo_blocks = [b for b in range(FF // 128) if b not in vblocks]

    def start_piece(q):
        hi_wd(q, *issue[q]).start(priority=HI)

    def wait_piece(q):
        hi_wd(q, *issue[q]).wait()
        waited.add(q)
        have.add(wd_piece(q))

    def vpu_piece(acc, q):
        p = wd_piece(q)
        if p // 8 not in vblocks:
            return acc
        c0 = 256 + vblocks.index(p // 8) * 128 + (p % 8) * 16
        return vpu_rows(acc, wd_v[p * 16:(p + 1) * 16, :], c0, 16)

    row8 = lax.broadcasted_iota(jnp.int32, (8, D), 0)
    acc = jnp.where(row8 == 0, x + xn, 0.0)
    for c in range(N4 - 1):
        it = BASE[4] + c
        starts = [q for q, (i, _) in issue.items() if i == it]
        waits = [q for q, (i, _) in issue.items() if i == it - AH]
        low(4, c).wait()
        for q in starts[:1]:
            start_piece(q)
        if c + AL < N4 - 1:
            low(4, c + AL).start(priority=LO)
        elif c + AL == N4 - 1:
            for i in range(len(SUB)):
                sub(i).start(priority=LO)
        l = jnp.where(row2 == c // 4, lhs[c % 4], 0.0).astype(BF16)
        acc = acc + jnp.dot(l, wo_v[c].reshape(2 * DH, D), preferred_element_type=F32)
        for q in waits[:-1]:
            wait_piece(q)
        for q in starts[1:2]:
            start_piece(q)
        ready = [b for b in todo_blocks if all(p in have for p in range(8 * b, 8 * b + 8))]
        for b in ready[:1]:
            todo_blocks.remove(b)
            acc = acc + jnp.dot(hb[:, b * 128:(b + 1) * 128], wd_v[b * 128:(b + 1) * 128, :],
                                preferred_element_type=F32)
        for slot in range(4):
            if TOCOL[slot] == c:
                if slot < 2:
                    to_col(slot, lhs[3][rep - 1:rep, slot * 128:(slot + 1) * 128])
                else:
                    b = vblocks[slot - 2]
                    to_col(slot, hid[:, b * 128:(b + 1) * 128])
        for q in waits[-1:]:
            wait_piece(q)
        for q in starts[2:3]:
            start_piece(q)
        for q in waits:
            assert wd_piece(q) // 8 not in vblocks or c > max(TOCOL[2:])
            acc = vpu_piece(acc, q)
        for q in starts[3:]:
            start_piece(q)
    assert not todo_blocks
    rest = [q for q in range(NWD) if q not in waited]
    last_it = max(issue[q][0] for q in rest)
    for q in rest:
        if issue[q][0] != last_it:
            wait_piece(q)
            acc = vpu_piece(acc, q)
    for i in range(len(SUB)):
        if i == LATE_POS:
            late = [q for q in rest if issue[q][0] == last_it]
            for q in late:
                wait_piece(q)
            for q in late:
                acc = vpu_piece(acc, q)
        g0, ng, r0, nr = SUB[i]
        sub(i).wait()
        for gi in range(g0, g0 + ng):
            acc = vpu_rows(acc, wo_v[N4 - 1, gi, r0:r0 + nr, :], gi * 32 + r0, nr)
    out_ref[0] = jnp.sum(acc, axis=0, keepdims=True).astype(out_ref.dtype)


@jax.jit
def pallas_parallel_sum__sliding_block_cached__moe_arch_mod__decode_kernel(
    A_x: jax.Array,
    A_k_cache: jax.Array,
    A_v_cache: jax.Array,
    A_wq: jax.Array,
    A_wo: jax.Array,
    B_x: jax.Array,
    B_w_r: jax.Array,
    B_w_gate: jax.Array,
    B_w_up: jax.Array,
    B_w_down: jax.Array,
):
    del B_x
    hkv, sk = A_k_cache.shape[1], A_k_cache.shape[2]
    W = min(4096, max(256, sk // 4))
    D = A_x.shape[-1]
    FF = B_w_gate.shape[1]
    nkc = W // 128
    wq3 = A_wq.reshape(NG, D // NG, HQ * DH)
    wo3 = A_wo.reshape(NG, HQ * DH // NG, D)
    anyspec = pl.BlockSpec(memory_space=pl.ANY)
    return pl.pallas_call(
        _kernel,
        out_shape=jax.ShapeDtypeStruct(A_x.shape, A_x.dtype),
        in_specs=[anyspec] * 9,
        out_specs=pl.BlockSpec(memory_space=pltpu.VMEM),
        scratch_shapes=[
            pltpu.VMEM(A_x.shape, BF16), pltpu.VMEM(B_w_r.shape, BF16),
            pltpu.VMEM((16, NG, 8, HQ * DH // 2), BF16),
            pltpu.VMEM((nkc, hkv, 128, DH), BF16), pltpu.VMEM((nkc, hkv, 128, DH), BF16),
            pltpu.VMEM((16, NG, 32, D), BF16),
            pltpu.VMEM((2 * nkc, 4, 8, FF // 2), BF16), pltpu.VMEM(B_w_down.shape, BF16),
            pltpu.VMEM((D, 128), F32), pltpu.VMEM((2, 8, HQ * DH // 2), F32),
            pltpu.VMEM((2, 2, 8, FF // 2), F32),
            pltpu.VMEM((hkv, 8, DH), F32), pltpu.VMEM((nkc, hkv, 8, DH), F32),
            pltpu.VMEM((hkv, 8, DH), F32),
            pltpu.VMEM((512, 128), F32),
            pltpu.SemaphoreType.DMA((NS,)), pltpu.SemaphoreType.DMA((NS * 4,)),
            pltpu.SemaphoreType.DMA((2 + len(SUB),)),
        ],
        compiler_params=pltpu.CompilerParams(
            vmem_limit_bytes=48 * 1024 * 1024,
            disable_semaphore_checks=True,
        ),
    )(A_x, A_k_cache, A_v_cache, wq3, wo3, B_w_r, B_w_gate, B_w_up, B_w_down)
```

```python
import jax
import jax.numpy as jnp
from jax import lax
import jax.experimental.pallas as pl
import jax.experimental.pallas.tpu as pltpu

HQ, DH = 32, 128
F32 = jnp.float32
BF16 = jnp.bfloat16
NT = (((1,), (1,)), ((), ()))
NG = 8
LO, HI = 1, 0
NS = 8
AL = 5
AH = 4
P4HI = (4,) + (3,) * 12
SUB = ((0, 4, 0, 32), (4, 2, 0, 32), (6, 1, 0, 32), (7, 1, 0, 16), (7, 1, 16, 16))
LATE_POS = 1
TOCOL = (8, 9, 6, 7)
SH = 16


def _kernel(x_hbm, k_hbm, v_hbm, wq_hbm, wo_hbm, wr_hbm, wg_hbm, wu_hbm, wd_hbm, out_ref,
            x_v, wr_v, wq_v, k_v, v_v, wo_v, gu_v, wd_v,
            xcol, qacc, guacc, q_s, s_s, m_s, col_s, lsem, hsem, msem):
    hkv, sk = k_hbm.shape[1], k_hbm.shape[2]
    nkc = k_v.shape[0]
    W = nkc * 128
    D = x_v.shape[-1]
    FF = wg_hbm.shape[1]
    rep = HQ // hkv
    HF = FF // 2
    QH = (HQ * DH) // 2
    N1, N2, N3, N4 = 16, nkc, nkc, 16
    BASE = {1: 0, 2: N1, 3: N1 + N2, 4: N1 + N2 + N3}
    NP = {1: N1, 2: N2, 3: N3, 4: N4}
    NWD = FF // 16
    WD_P3 = 4 * (N1 - AH + 2)
    WD_P4 = WD_P3 + 4 * AH
    assert WD_P4 + sum(P4HI) == NWD and hkv == NG and rep == 4 and D == 16 * nkc

    def mo(i, m):
        return i if isinstance(i, int) else pl.multiple_of(i, m)

    def low(p, s):
        if p == 1:
            r, hf = s // 2, s % 2
            src = wq_hbm.at[:, pl.ds(mo(r * 8, 8), 8), pl.ds(mo(hf * QH, 128), QH)]
            dst = wq_v.at[s]
        elif p in (2, 3):
            h, v = (k_hbm, k_v) if p == 2 else (v_hbm, v_v)
            src, dst = h.at[0, :, pl.ds(mo(sk - W - SH + s * 128, 16), 128)], v.at[s]
        else:
            src, dst = wo_hbm.at[:, pl.ds(mo(s * 32, 32), 32)], wo_v.at[s]
        return pltpu.make_async_copy(src, dst, lsem.at[(BASE[p] + s) % NS])

    def low0(p, part):
        h, v = (k_hbm, k_v) if p == 2 else (v_hbm, v_v)
        if part == 0:
            return pltpu.make_async_copy(h.at[0, :, pl.ds(sk - W, 128 - SH)],
                                         v.at[0, :, pl.ds(SH, 128 - SH)], lsem.at[BASE[p] % NS])
        return pltpu.make_async_copy(h.at[0, :, pl.ds(sk - SH, SH)],
                                     v.at[0, :, pl.ds(0, SH)], msem.at[p - 2])

    def sub(i):
        g0, ng, r0, nr = SUB[i]
        s = N4 - 1
        return pltpu.make_async_copy(wo_hbm.at[pl.ds(g0, ng), pl.ds(s * 32 + r0, nr)],
                                     wo_v.at[s, pl.ds(g0, ng), pl.ds(r0, nr)], msem.at[2 + i])

    def hsem_at(it, k):
        return hsem.at[((it + 2) % NS) * 4 + k]

    def wd_piece(seq):
        return (seq % 2) * (NWD // 2) + seq // 2

    def hi_wd(seq, it, k):
        sl = pl.ds(mo(wd_piece(seq) * 16, 16), 16)
        return pltpu.make_async_copy(wd_hbm.at[sl], wd_v.at[sl], hsem_at(it, k))

    def gu_row(u, k):
        return mo((u // 2 + (k // 2) * (D // 16)) * 8, 8)

    def hi_gu(u, k):
        h = wg_hbm if k % 2 == 0 else wu_hbm
        src = h.at[pl.ds(gu_row(u, k), 8), pl.ds(mo((u % 2) * HF, 128), HF)]
        return pltpu.make_async_copy(src, gu_v.at[u, k], hsem_at(N1 + u - AH, k))

    def branch(cond, fa, fb):
        pl.when(cond)(fa)
        pl.when(jnp.logical_not(cond))(fb)

    def start_low(p, s):
        n = NP[p]
        pl.when(s + AL < n)(lambda: low(p, s + AL).start(priority=LO))
        if p < 3:
            @pl.when(s + AL == n)
            def _():
                low0(p + 1, 0).start(priority=LO)
                low0(p + 1, 1).start(priority=LO)
            pl.when(s + AL > n)(lambda: low(p + 1, s + AL - n).start(priority=LO))
        else:
            pl.when(s + AL >= n)(lambda: low(p + 1, s + AL - n).start(priority=LO))

    def wait_low(p, c):
        @pl.when(c == 0)
        def _():
            low0(p, 0).wait()
            low0(p, 1).wait()
        pl.when(c > 0)(lambda: low(p, c).wait())

    def start_high(p, s, k):
        n, it = NP[p], BASE[p] + s

        def gu():
            hi_gu(it + AH - N1, k).start(priority=HI)

        if p == 1:
            branch(s + AH < n, lambda: hi_wd(4 * (s + 2) + k, it, k).start(priority=HI), gu)
        elif p == 2:
            gu()
        else:
            branch(s + AH < n, gu, lambda: hi_wd(WD_P3 + 4 * (s + AH - n) + k, it, k).start(priority=HI))

    cp_x = pltpu.make_async_copy(x_hbm, x_v, msem.at[0])
    cp_wr = pltpu.make_async_copy(wr_hbm, wr_v, msem.at[1])

    cp_x.start(priority=HI)
    low(1, 0).start(priority=LO)
    cp_wr.start(priority=HI)
    for s in range(1, AL):
        low(1, s).start(priority=LO)

    def fill(k, carry):
        hi_wd(k, -2, k).start(priority=HI)
        s_s[pl.ds(k * (nkc // 4), nkc // 4)] = jnp.zeros((nkc // 4,) + s_s.shape[1:], F32)
        return carry
    lax.fori_loop(0, 4, fill, 0)

    cp_x.wait()
    hi_wd(4, -1, 0).start(priority=HI)
    x = x_v[0].astype(F32)
    mu = jnp.mean(x, axis=-1, keepdims=True)
    xc = x - mu
    var = jnp.mean(xc * xc, axis=-1, keepdims=True)
    xn = xc / jnp.sqrt(var + 1e-5)
    qacc[...] = jnp.zeros(qacc.shape, F32)
    guacc[...] = jnp.zeros(guacc.shape, F32)
    cp_wr.wait()
    hi_wd(5, -1, 1).start(priority=HI)
    for b in range(D // 128):
        xcol[b * 128:(b + 1) * 128, :] = jnp.transpose(
            jnp.broadcast_to(xn[:, b * 128:(b + 1) * 128], (128, 128)))
        if b % 2 == 1:
            hi_wd(b - 1, -2, b - 1).wait()
            hi_wd(b, -2, b).wait()
            hi_wd(6 + b // 2, -1, 2 + b // 2).start(priority=HI)
    wr = wr_v[...].astype(F32).reshape(1, D)
    gate = jax.nn.sigmoid(jnp.sum(xn * wr, axis=-1, keepdims=True))

    def lanes(col, n):
        return jnp.concatenate([col] * n, axis=1)

    def p1(r, carry):
        for hf in range(2):
            s = r * 2 + hf
            low(1, s).wait()
            for k in range(4):
                @pl.when(s >= AH - 1)
                def _():
                    hi_wd(4 * (s - AH + 2) + k, s - AH, k).wait()
                start_high(1, s, k)
                if k == 0:
                    start_low(1, s)
                acc = qacc[hf, :, k * 512:(k + 1) * 512]
                for g in range(NG):
                    xc8 = xcol[pl.ds(pl.multiple_of(g * 64 + r * 8, 8), 8), :]
                    acc = acc + wq_v[s, g, :, k * 512:(k + 1) * 512].astype(F32) * lanes(xc8, 4)
                qacc[hf, :, k * 512:(k + 1) * 512] = acc
        return carry
    lax.fori_loop(0, N1 // 2, p1, 0)

    row = lax.broadcasted_iota(jnp.int32, (8, DH), 0)
    for h in range(hkv):
        qh = None
        for j in range(rep):
            n = h * rep + j
            qn = jnp.sum(qacc[n // 16, :, (n % 16) * DH:(n % 16 + 1) * DH], axis=0, keepdims=True)
            qn = jnp.broadcast_to(qn, (8, DH))
            qh = qn if qh is None else jnp.where(row == j, qn, qh)
        q_s[h] = qh * (DH ** -0.5)

    def ffn_part(u, w):
        acc = guacc[w, u % 2]
        for k in (w, w + 2):
            acc = acc + gu_v[u, k].astype(F32) * lanes(xcol[pl.ds(gu_row(u, k), 8), :], HF // 128)
        guacc[w, u % 2] = acc

    def step23(p, c, heads):
        u = BASE[p] - N1 + c
        wait_low(p, c)
        start_high(p, c, 0)
        start_low(p, c)
        heads(range(0, 4))
        hi_gu(u, 0).wait()
        hi_gu(u, 2).wait()
        start_high(p, c, 1)
        ffn_part(u, 0)
        hi_gu(u, 1).wait()
        start_high(p, c, 2)
        heads(range(4, 8))
        hi_gu(u, 3).wait()
        start_high(p, c, 3)
        ffn_part(u, 1)

    def p2(c, ms):
        ms = list(ms)

        def heads(hs):
            for h in hs:
                s = lax.dot_general(q_s[h].astype(BF16), k_v[c, h], NT, preferred_element_type=F32)
                s_s[c, h] = s
                ms[h] = jnp.maximum(ms[h], s)
        step23(2, c, heads)
        return tuple(ms)
    neg = jnp.full((8, DH), -jnp.inf, F32)
    ms = lax.fori_loop(0, N2, p2, (neg,) * hkv)
    for h in range(hkv):
        m_s[h] = jnp.broadcast_to(jnp.max(ms[h], axis=-1, keepdims=True), (8, DH))

    def p3(c, carry):
        os_, ls = list(carry[0]), list(carry[1])

        def heads(hs):
            for h in hs:
                p = jnp.exp(s_s[c, h] - m_s[h])
                ls[h] = ls[h] + p
                os_[h] = os_[h] + jnp.dot(p.astype(BF16), v_v[c, h], preferred_element_type=F32)
        step23(3, c, heads)
        return tuple(os_), tuple(ls)
    zero = jnp.zeros((8, DH), F32)
    os_, ls = lax.fori_loop(0, N3, p3, ((zero,) * hkv, (zero,) * hkv))

    on = [os_[h] / jnp.sum(ls[h], axis=-1, keepdims=True) for h in range(hkv)]
    lhs = [jnp.concatenate([on[h][:, q * 32:(q + 1) * 32] for h in range(hkv)], axis=1) for q in range(4)]
    row2 = lax.broadcasted_iota(jnp.int32, (8, 2 * DH), 0)
    g, up = [jnp.concatenate([jnp.sum(guacc[w, hf], axis=0, keepdims=True) for hf in range(2)], axis=1)
             for w in range(2)]
    hid = g * jax.nn.sigmoid(g) * up * gate
    rowf = lax.broadcasted_iota(jnp.int32, (8, FF), 0)
    hb = jnp.where(rowf == 0, hid, 0.0).astype(BF16)

    def to_col(slot, vec):
        col_s[slot * 128:(slot + 1) * 128, :] = jnp.transpose(jnp.broadcast_to(vec, (128, 128)))

    def vpu_rows(acc, w, c0, n):
        prod = w.astype(F32) * lanes(col_s[c0:c0 + n, :], D // 128)
        return acc + jnp.sum(prod.reshape(n // 8, 8, D), axis=0)

    issue = {}
    for j in range(AH):
        for k in range(4):
            issue[WD_P3 + 4 * j + k] = (BASE[4] - AH + j, k)
    pc = WD_P4
    for c, cnt in enumerate(P4HI):
        for k in range(cnt):
            issue[pc] = (BASE[4] + c, k)
            pc += 1
    vblocks = sorted({wd_piece(q) // 8 for q in range(NWD - 16, NWD)})
    assert len(vblocks) == 2
    have = {wd_piece(q) for q in range(WD_P3)}
    waited = set(range(WD_P3))
    todo_blocks = [b for b in range(FF // 128) if b not in vblocks]

    def start_piece(q):
        hi_wd(q, *issue[q]).start(priority=HI)

    def wait_piece(q):
        hi_wd(q, *issue[q]).wait()
        waited.add(q)
        have.add(wd_piece(q))

    def vpu_piece(acc, q):
        p = wd_piece(q)
        if p // 8 not in vblocks:
            return acc
        c0 = 256 + vblocks.index(p // 8) * 128 + (p % 8) * 16
        return vpu_rows(acc, wd_v[p * 16:(p + 1) * 16, :], c0, 16)

    row8 = lax.broadcasted_iota(jnp.int32, (8, D), 0)
    acc = jnp.where(row8 == 0, x + xn, 0.0)
    for c in range(N4 - 1):
        it = BASE[4] + c
        starts = [q for q, (i, _) in issue.items() if i == it]
        waits = [q for q, (i, _) in issue.items() if i == it - AH]
        low(4, c).wait()
        for q in starts[:1]:
            start_piece(q)
        if c + AL < N4 - 1:
            low(4, c + AL).start(priority=LO)
        elif c + AL == N4 - 1:
            for i in range(len(SUB)):
                sub(i).start(priority=LO)
        l = jnp.where(row2 == c // 4, lhs[c % 4], 0.0).astype(BF16)
        acc = acc + jnp.dot(l, wo_v[c].reshape(2 * DH, D), preferred_element_type=F32)
        for q in waits[:-1]:
            wait_piece(q)
        for q in starts[1:2]:
            start_piece(q)
        ready = [b for b in todo_blocks if all(p in have for p in range(8 * b, 8 * b + 8))]
        for b in ready[:1]:
            todo_blocks.remove(b)
            acc = acc + jnp.dot(hb[:, b * 128:(b + 1) * 128], wd_v[b * 128:(b + 1) * 128, :],
                                preferred_element_type=F32)
        for slot in range(4):
            if TOCOL[slot] == c:
                if slot < 2:
                    to_col(slot, lhs[3][rep - 1:rep, slot * 128:(slot + 1) * 128])
                else:
                    b = vblocks[slot - 2]
                    to_col(slot, hid[:, b * 128:(b + 1) * 128])
        for q in waits[-1:]:
            wait_piece(q)
        for q in starts[2:3]:
            start_piece(q)
        for q in waits:
            assert wd_piece(q) // 8 not in vblocks or c > max(TOCOL[2:])
            acc = vpu_piece(acc, q)
        for q in starts[3:]:
            start_piece(q)
    assert not todo_blocks
    rest = [q for q in range(NWD) if q not in waited]
    last_it = max(issue[q][0] for q in rest)
    for q in rest:
        if issue[q][0] != last_it:
            wait_piece(q)
            acc = vpu_piece(acc, q)
    for i in range(len(SUB)):
        if i == LATE_POS:
            late = [q for q in rest if issue[q][0] == last_it]
            for q in late:
                wait_piece(q)
            for q in late:
                acc = vpu_piece(acc, q)
        g0, ng, r0, nr = SUB[i]
        sub(i).wait()
        for gi in range(g0, g0 + ng):
            acc = vpu_rows(acc, wo_v[N4 - 1, gi, r0:r0 + nr, :], gi * 32 + r0, nr)
    out_ref[0] = jnp.sum(acc, axis=0, keepdims=True).astype(out_ref.dtype)


@jax.jit
def pallas_parallel_sum__sliding_block_cached__moe_arch_mod__decode_kernel(
    A_x: jax.Array,
    A_k_cache: jax.Array,
    A_v_cache: jax.Array,
    A_wq: jax.Array,
    A_wo: jax.Array,
    B_x: jax.Array,
    B_w_r: jax.Array,
    B_w_gate: jax.Array,
    B_w_up: jax.Array,
    B_w_down: jax.Array,
):
    del B_x
    hkv, sk = A_k_cache.shape[1], A_k_cache.shape[2]
    W = min(4096, max(256, sk // 4))
    D = A_x.shape[-1]
    FF = B_w_gate.shape[1]
    nkc = W // 128
    wq3 = A_wq.reshape(NG, D // NG, HQ * DH)
    wo3 = A_wo.reshape(NG, HQ * DH // NG, D)
    anyspec = pl.BlockSpec(memory_space=pl.ANY)
    return pl.pallas_call(
        _kernel,
        out_shape=jax.ShapeDtypeStruct(A_x.shape, A_x.dtype),
        in_specs=[anyspec] * 9,
        out_specs=pl.BlockSpec(memory_space=pltpu.VMEM),
        scratch_shapes=[
            pltpu.VMEM(A_x.shape, BF16), pltpu.VMEM(B_w_r.shape, BF16),
            pltpu.VMEM((16, NG, 8, HQ * DH // 2), BF16),
            pltpu.VMEM((nkc, hkv, 128, DH), BF16), pltpu.VMEM((nkc, hkv, 128, DH), BF16),
            pltpu.VMEM((16, NG, 32, D), BF16),
            pltpu.VMEM((2 * nkc, 4, 8, FF // 2), BF16), pltpu.VMEM(B_w_down.shape, BF16),
            pltpu.VMEM((D, 128), F32), pltpu.VMEM((2, 8, HQ * DH // 2), F32),
            pltpu.VMEM((2, 2, 8, FF // 2), F32),
            pltpu.VMEM((hkv, 8, DH), F32), pltpu.VMEM((nkc, hkv, 8, DH), F32),
            pltpu.VMEM((hkv, 8, DH), F32),
            pltpu.VMEM((512, 128), F32),
            pltpu.SemaphoreType.DMA((NS,)), pltpu.SemaphoreType.DMA((NS * 4,)),
            pltpu.SemaphoreType.DMA((2 + len(SUB),)),
        ],
        compiler_params=pltpu.CompilerParams(
            vmem_limit_bytes=48 * 1024 * 1024,
            disable_semaphore_checks=True,
        ),
    )(A_x, A_k_cache, A_v_cache, wq3, wo3, B_w_r, B_w_gate, B_w_up, B_w_down)
```

```python
import jax
import jax.numpy as jnp
from jax import lax
import jax.experimental.pallas as pl
import jax.experimental.pallas.tpu as pltpu

HQ, DH = 32, 128
F32 = jnp.float32
BF16 = jnp.bfloat16
NT = (((1,), (1,)), ((), ()))
NG = 8
LO, HI = 1, 0
NS = 8
CH = 256
SH = 144
AL = 5
AH = 4
P4HI = (4,) + (3,) * 12
SUB = ((4, 2, 0, 256), (6, 1, 0, 256), (7, 1, 0, 128), (7, 1, 128, 64), (7, 1, 192, 64))
LATE_POS = 1
TOCOL = (8, 9, 10, 11, 6, 7)


def _kernel(x_hbm, k_hbm, v_hbm, wq_hbm, wo_hbm, wr_hbm, wg_hbm, wu_hbm, wd_hbm, out_ref,
            x_v, wr_v, wq_v, k_v, v_v, wo_v, gu_v, wd_v,
            xcol, qacc, guacc, q_s, s_s, m_s, col_s, e_s, ex_s, lsem, hsem, msem):
    hkv, sk = k_hbm.shape[1], k_hbm.shape[2]
    W = k_v.shape[0] * CH
    D = x_v.shape[-1]
    FF = wg_hbm.shape[1]
    rep = HQ // hkv
    HF = FF // 2
    N1, N2, N3, N4 = 16, 2 * W // CH, 2 * W // CH, 16
    BASE = {1: 0, 2: N1, 3: N1 + N2, 4: N1 + N2 + N3}
    NP = {1: N1, 2: N2, 3: N3, 4: N4}
    NWD = FF // 16
    WD_P3 = 4 * (N1 - AH + 2)
    WD_P4 = WD_P3 + 4 * AH
    ST = SH // 8
    assert WD_P4 + sum(P4HI) == NWD and hkv == NG and rep == 4 and D == 4 * DH and N2 + N3 == D // 8
    stream = {1: (wq_hbm, wq_v, 0), 2: (k_hbm.at[0], k_v, sk - W),
              3: (v_hbm.at[0], v_v, sk - W), 4: (wo_hbm, wo_v, 0)}

    def mo(i, m):
        return i if isinstance(i, int) else pl.multiple_of(i, m)

    def low(p, c, t):
        h, v, lo = stream[p]
        gs = pl.ds(4 * t, 4)
        return pltpu.make_async_copy(h.at[gs, pl.ds(mo(lo - SH + c * CH, 16), CH)], v.at[c, gs],
                                     lsem.at[(BASE[p] + 2 * c + t) % NS])

    def low0(p, t, part):
        h, v, lo = stream[p]
        gs = pl.ds(4 * t, 4)
        if part == 0:
            return pltpu.make_async_copy(h.at[gs, pl.ds(lo, CH - SH)], v.at[0, gs, pl.ds(SH, CH - SH)],
                                         lsem.at[(BASE[p] + t) % NS])
        hi = lo + v.shape[0] * CH
        return pltpu.make_async_copy(h.at[gs, pl.ds(hi - SH, SH)], v.at[0, gs, pl.ds(0, SH)],
                                     msem.at[2 + t])

    def go(cp):
        cp.start(priority=LO)

    def wait(cp):
        cp.wait()

    def low_do(p, c, t, act):
        def first():
            act(low0(p, t, 0))
            act(low0(p, t, 1))

        def other():
            act(low(p, c, t))

        if isinstance(c, int):
            (first if c == 0 else other)()
        else:
            pl.when(c == 0)(first)
            pl.when(c > 0)(other)

    def sub(i):
        g0, ng, r0, nr = SUB[i]
        c = N4 // 2 - 1
        return pltpu.make_async_copy(wo_hbm.at[pl.ds(g0, ng), pl.ds(c * CH - SH + r0, nr)],
                                     wo_v.at[c, pl.ds(g0, ng), pl.ds(r0, nr)], msem.at[4 + i])

    def hsem_at(it, k):
        return hsem.at[((it + 2) % NS) * 4 + k]

    def wd_piece(seq):
        return (seq % 2) * (NWD // 2) + seq // 2

    def hi_wd(seq, it, k):
        sl = pl.ds(mo(wd_piece(seq) * 16, 16), 16)
        return pltpu.make_async_copy(wd_hbm.at[sl], wd_v.at[sl], hsem_at(it, k))

    def gu_row(u, k):
        return mo((u // 2 + (k // 2) * (D // 16)) * 8, 8)

    def hi_gu(u, k):
        h = wg_hbm if k % 2 == 0 else wu_hbm
        src = h.at[pl.ds(gu_row(u, k), 8), pl.ds(mo((u % 2) * HF, 128), HF)]
        return pltpu.make_async_copy(src, gu_v.at[u, k], hsem_at(N1 + u - AH, k))

    def branch(cond, fa, fb):
        pl.when(cond)(fa)
        pl.when(jnp.logical_not(cond))(fb)

    def start_low(p, c, t):
        nc = NP[p] // 2
        c2, t2 = c + (t + AL) // 2, (t + AL) % 2
        pl.when(c2 < nc)(lambda: go(low(p, c2, t2)))
        pl.when(c2 == nc)(lambda: low_do(p + 1, 0, t2, go))
        pl.when(c2 > nc)(lambda: go(low(p + 1, c2 - nc, t2)))

    def start_high(p, s, k):
        n, it = NP[p], BASE[p] + s

        def gu():
            hi_gu(it + AH - N1, k).start(priority=HI)

        if p == 1:
            branch(s + AH < n, lambda: hi_wd(4 * (s + 2) + k, it, k).start(priority=HI), gu)
        elif p == 2:
            gu()
        else:
            branch(s + AH < n, gu, lambda: hi_wd(WD_P3 + 4 * (s + AH - n) + k, it, k).start(priority=HI))

    cp_x = pltpu.make_async_copy(x_hbm, x_v, msem.at[0])
    cp_wr = pltpu.make_async_copy(wr_hbm, wr_v, msem.at[1])

    cp_x.start(priority=HI)
    low_do(1, 0, 0, go)
    cp_wr.start(priority=HI)
    for s in range(1, AL):
        low_do(1, s // 2, s % 2, go)

    def fill(k, carry):
        hi_wd(k, -2, k).start(priority=HI)
        d = lax.broadcasted_iota(jnp.int32, (64, D), 0) + k * 64
        p = lax.broadcasted_iota(jnp.int32, (64, D), 1)
        f = p - SH + jnp.where(p < SH, 2 * D, 0)
        e = jnp.where(d == (f // 32) * 8 + f % 8, 1.0, 0.0)
        e_s[pl.ds(pl.multiple_of(k * 64, 64), 64), :] = e.astype(BF16)
        return carry
    lax.fori_loop(0, 4, fill, 0)

    cp_x.wait()
    hi_wd(4, -1, 0).start(priority=HI)
    x = x_v[0].astype(F32)
    mu = jnp.mean(x, axis=-1, keepdims=True)
    xc = x - mu
    var = jnp.mean(xc * xc, axis=-1, keepdims=True)
    xn = xc / jnp.sqrt(var + 1e-5)
    qacc[...] = jnp.zeros(qacc.shape, F32)
    guacc[...] = jnp.zeros(guacc.shape, F32)
    cp_wr.wait()
    hi_wd(5, -1, 1).start(priority=HI)
    for b in range(D // 128):
        xcol[b * 128:(b + 1) * 128, :] = jnp.transpose(
            jnp.broadcast_to(xn[:, b * 128:(b + 1) * 128], (128, 128)))
        if b % 2 == 1:
            hi_wd(b - 1, -2, b - 1).wait()
            hi_wd(b, -2, b).wait()
            hi_wd(6 + b // 2, -1, 2 + b // 2).start(priority=HI)
    wr = wr_v[...].astype(F32).reshape(1, D)
    gate = jax.nn.sigmoid(jnp.sum(xn * wr, axis=-1, keepdims=True))

    def lanes(col, n):
        return jnp.concatenate([col] * n, axis=1)

    def p1(c, carry):
        for t in range(2):
            s = 2 * c + t
            low_do(1, c, t, wait)
            for k in range(4):
                @pl.when(s >= AH - 1)
                def _():
                    hi_wd(4 * (s - AH + 2) + k, s - AH, k).wait()
                start_high(1, s, k)
                if k == 0:
                    start_low(1, c, t)
                acc = qacc[8 * k:8 * k + 8]
                for g in range(4 * t, 4 * t + 4):
                    xcur = xcol[pl.ds(pl.multiple_of(g * 64 + c * 8, 8), 8), :]
                    xprv = xcol[pl.ds(pl.multiple_of(g * 64 + ((c + 7) % 8) * 8, 8), 8), :]
                    xs = jnp.concatenate([xprv if tau < ST else xcur for tau in range(8 * k, 8 * k + 8)],
                                         axis=0)
                    acc = acc + (wq_v[c, g, k * 64:(k + 1) * 64, :].astype(F32) * xs).reshape(8, 8, DH)
                qacc[8 * k:8 * k + 8] = acc
        return carry
    lax.fori_loop(0, N1 // 2, p1, 0)

    row = lax.broadcasted_iota(jnp.int32, (8, DH), 0)
    for h in range(hkv):
        qh = None
        for j in range(rep):
            qn = jnp.sum(qacc[(h * rep + j + ST) % HQ], axis=0, keepdims=True)
            qn = jnp.broadcast_to(qn, (8, DH))
            qh = qn if qh is None else jnp.where(row == j, qn, qh)
        q_s[h] = qh * (DH ** -0.5)

    def ffn_part(u, half, w):
        acc = guacc[w, half]
        for k in (w, w + 2):
            acc = acc + gu_v[u, k].astype(F32) * lanes(xcol[pl.ds(gu_row(u, k), 8), :], HF // 128)
        guacc[w, half] = acc

    def step23(p, c, t, heads):
        s = 2 * c + t
        u = BASE[p] - N1 + s
        low_do(p, c, t, wait)
        start_high(p, s, 0)
        start_low(p, c, t)
        heads(range(4 * t, 4 * t + 2))
        hi_gu(u, 0).wait()
        hi_gu(u, 2).wait()
        start_high(p, s, 1)
        ffn_part(u, t, 0)
        hi_gu(u, 1).wait()
        start_high(p, s, 2)
        heads(range(4 * t + 2, 4 * t + 4))
        hi_gu(u, 3).wait()
        start_high(p, s, 3)
        ffn_part(u, t, 1)

    def p2(c, ms):
        ms = list(ms)

        def heads(hs):
            for h in hs:
                s = lax.dot_general(q_s[h].astype(BF16), k_v[c, h], NT, preferred_element_type=F32)
                s_s[c, h] = s
                ms[h] = jnp.maximum(ms[h], jnp.maximum(s[:, :DH], s[:, DH:]))
        for t in range(2):
            step23(2, c, t, heads)
        return tuple(ms)
    neg = jnp.full((8, DH), -jnp.inf, F32)
    ms = lax.fori_loop(0, N2 // 2, p2, (neg,) * hkv)
    for h in range(hkv):
        m_s[h] = jnp.broadcast_to(jnp.max(ms[h], axis=-1, keepdims=True), (8, DH))

    def p3(c, carry):
        os_, ls = list(carry[0]), list(carry[1])

        def heads(hs):
            for h in hs:
                p = jnp.exp(s_s[c, h] - lanes(m_s[h], 2))
                ls[h] = ls[h] + (p[:, :DH] + p[:, DH:])
                os_[h] = os_[h] + jnp.dot(p.astype(BF16), v_v[c, h], preferred_element_type=F32)
        for t in range(2):
            step23(3, c, t, heads)
        return tuple(os_), tuple(ls)
    zero = jnp.zeros((8, DH), F32)
    os_, ls = lax.fori_loop(0, N3 // 2, p3, ((zero,) * hkv, (zero,) * hkv))

    on = [os_[h] / jnp.sum(ls[h], axis=-1, keepdims=True) for h in range(hkv)]
    both = [jnp.concatenate([o, jnp.concatenate([o[rep - 1:rep], o[:rep - 1], o[rep:]], axis=0)], axis=1)
            for o in on]
    ex_s[...] = jnp.dot(jnp.concatenate(both, axis=0).astype(BF16), e_s[...], preferred_element_type=F32)
    pos = lax.broadcasted_iota(jnp.int32, (8, CH), 1)
    ctmask = lax.broadcasted_iota(jnp.int32, (8, CH), 0) == (pos // 8 + (-ST) % 4) % 4
    g, up = [jnp.concatenate([jnp.sum(guacc[w, hf], axis=0, keepdims=True) for hf in range(2)], axis=1)
             for w in range(2)]
    hid = g * jax.nn.sigmoid(g) * up * gate
    rowf = lax.broadcasted_iota(jnp.int32, (8, FF), 0)
    hb = jnp.where(rowf == 0, hid, 0.0).astype(BF16)

    def to_col(slot, vec):
        col_s[slot * 128:(slot + 1) * 128, :] = jnp.transpose(jnp.broadcast_to(vec, (128, 128)))

    issue = {}
    for j in range(AH):
        for k in range(4):
            issue[WD_P3 + 4 * j + k] = (BASE[4] - AH + j, k)
    pc = WD_P4
    for s, cnt in enumerate(P4HI):
        for k in range(cnt):
            issue[pc] = (BASE[4] + s, k)
            pc += 1
    vblocks = sorted({wd_piece(q) // 8 for q in range(NWD - 16, NWD)})
    assert len(vblocks) == 2
    have = {wd_piece(q) for q in range(WD_P3)}
    waited = set(range(WD_P3))
    todo_blocks = [b for b in range(FF // 128) if b not in vblocks]

    def start_piece(q):
        hi_wd(q, *issue[q]).start(priority=HI)

    def wait_piece(q):
        hi_wd(q, *issue[q]).wait()
        waited.add(q)
        have.add(wd_piece(q))

    def vpu_piece(acc, q):
        p = wd_piece(q)
        if p // 8 not in vblocks:
            return acc
        c0 = (4 + vblocks.index(p // 8)) * 128 + (p % 8) * 16
        prod = wd_v[p * 16:(p + 1) * 16, :].astype(F32) * lanes(col_s[c0:c0 + 16, :], D // 128)
        return acc + jnp.sum(prod.reshape(2, 8, D), axis=0)

    def vpu_wo(acc, gi, r0, nr):
        c = N4 // 2 - 1
        cols = []
        for tau in range(r0 // 8, (r0 + nr) // 8):
            rt = (c * CH // 8 - ST + tau) // 4
            assert rt // 16 == rep - 1
            d0 = (gi - 4) * 128 + (rt % 16) * 8
            cols.append(col_s[d0:d0 + 8, :])
        prod = wo_v[c, gi, r0:r0 + nr, :].astype(F32) * jnp.concatenate(cols, axis=0)
        part = jnp.sum(prod.reshape(nr // 32, 4, 8, DH), axis=0)
        return acc + jnp.concatenate([part[(ct + ST) % 4] for ct in range(4)], axis=1)

    row8 = lax.broadcasted_iota(jnp.int32, (8, D), 0)
    acc = jnp.where(row8 == 0, x + xn, 0.0)
    accw = zero
    for s in range(N4 - 1):
        c, t = s // 2, s % 2
        it = BASE[4] + s
        starts = [q for q, (i, _) in issue.items() if i == it]
        waits = [q for q, (i, _) in issue.items() if i == it - AH]
        l = jnp.concatenate([
            jnp.where(ctmask, ex_s[8 * gi + c // 2:8 * gi + c // 2 + 1, (c % 2) * CH:(c % 2 + 1) * CH], 0.0)
            for gi in range(4 * t, 4 * t + 4)], axis=1).astype(BF16)
        low_do(4, c, t, wait)
        for q in starts[:1]:
            start_piece(q)
        if s + AL < N4 - 1:
            low_do(4, (s + AL) // 2, (s + AL) % 2, go)
        elif s + AL == N4 - 1:
            for i in range(len(SUB)):
                go(sub(i))
        accw = accw + jnp.dot(l, wo_v[c, 4 * t:4 * t + 4].reshape(4 * CH, DH), preferred_element_type=F32)
        for q in waits[:-1]:
            wait_piece(q)
        for q in starts[1:2]:
            start_piece(q)
        ready = [b for b in todo_blocks if all(p in have for p in range(8 * b, 8 * b + 8))]
        for b in ready[:1]:
            todo_blocks.remove(b)
            acc = acc + jnp.dot(hb[:, b * 128:(b + 1) * 128], wd_v[b * 128:(b + 1) * 128, :],
                                preferred_element_type=F32)
        for slot in range(6):
            if TOCOL[slot] == s:
                if slot < 4:
                    to_col(slot, on[4 + slot][rep - 1:rep, :])
                else:
                    b = vblocks[slot - 4]
                    to_col(slot, hid[:, b * 128:(b + 1) * 128])
        for q in waits[-1:]:
            wait_piece(q)
        for q in starts[2:3]:
            start_piece(q)
        for q in waits:
            assert wd_piece(q) // 8 not in vblocks or s > max(TOCOL[4:])
            acc = vpu_piece(acc, q)
        for q in starts[3:]:
            start_piece(q)
    assert not todo_blocks
    acc = acc + jnp.concatenate([jnp.where(row == ct, accw, 0.0) for ct in range(4)], axis=1)
    rest = [q for q in range(NWD) if q not in waited]
    last_it = max(issue[q][0] for q in rest)
    for q in rest:
        if issue[q][0] != last_it:
            wait_piece(q)
            acc = vpu_piece(acc, q)
    for i in range(len(SUB)):
        if i == LATE_POS:
            late = [q for q in rest if issue[q][0] == last_it]
            for q in late:
                wait_piece(q)
            for q in late:
                acc = vpu_piece(acc, q)
        g0, ng, r0, nr = SUB[i]
        sub(i).wait()
        for gi in range(g0, g0 + ng):
            acc = vpu_wo(acc, gi, r0, nr)
    out_ref[0] = jnp.sum(acc, axis=0, keepdims=True).astype(out_ref.dtype)


def _tiles(w):
    r, c = w.shape
    return w.reshape(r // 8, 8, c // 128, 128).transpose(0, 2, 1, 3).reshape(NG, -1, 128)


@jax.jit
def pallas_parallel_sum__sliding_block_cached__moe_arch_mod__decode_kernel(
    A_x: jax.Array,
    A_k_cache: jax.Array,
    A_v_cache: jax.Array,
    A_wq: jax.Array,
    A_wo: jax.Array,
    B_x: jax.Array,
    B_w_r: jax.Array,
    B_w_gate: jax.Array,
    B_w_up: jax.Array,
    B_w_down: jax.Array,
):
    del B_x
    hkv, sk = A_k_cache.shape[1], A_k_cache.shape[2]
    W = min(4096, max(256, sk // 4))
    D = A_x.shape[-1]
    FF = B_w_gate.shape[1]
    nkc = W // CH
    anyspec = pl.BlockSpec(memory_space=pl.ANY)
    return pl.pallas_call(
        _kernel,
        out_shape=jax.ShapeDtypeStruct(A_x.shape, A_x.dtype),
        in_specs=[anyspec] * 9,
        out_specs=pl.BlockSpec(memory_space=pltpu.VMEM),
        scratch_shapes=[
            pltpu.VMEM(A_x.shape, BF16), pltpu.VMEM(B_w_r.shape, BF16),
            pltpu.VMEM((8, NG, CH, DH), BF16),
            pltpu.VMEM((nkc, hkv, CH, DH), BF16), pltpu.VMEM((nkc, hkv, CH, DH), BF16),
            pltpu.VMEM((8, NG, CH, DH), BF16),
            pltpu.VMEM((4 * nkc, 4, 8, FF // 2), BF16), pltpu.VMEM(B_w_down.shape, BF16),
            pltpu.VMEM((D, 128), F32), pltpu.VMEM((HQ, 8, DH), F32), pltpu.VMEM((2, 2, 8, FF // 2), F32),
            pltpu.VMEM((hkv, 8, DH), F32), pltpu.VMEM((nkc, hkv, 8, CH), F32),
            pltpu.VMEM((hkv, 8, DH), F32),
            pltpu.VMEM((6 * 128, 128), F32), pltpu.VMEM((2 * DH, D), BF16), pltpu.VMEM((8 * hkv, D), F32),
            pltpu.SemaphoreType.DMA((NS,)), pltpu.SemaphoreType.DMA((NS * 4,)),
            pltpu.SemaphoreType.DMA((4 + len(SUB),)),
        ],
        compiler_params=pltpu.CompilerParams(
            vmem_limit_bytes=48 * 1024 * 1024,
            disable_semaphore_checks=True,
        ),
    )(A_x, A_k_cache, A_v_cache, _tiles(A_wq), _tiles(A_wo), B_w_r, B_w_gate, B_w_up, B_w_down)
```

```python
import jax
import jax.numpy as jnp
from jax import lax
import jax.experimental.pallas as pl
import jax.experimental.pallas.tpu as pltpu

HQ, DH = 32, 128
F32 = jnp.float32
BF16 = jnp.bfloat16
NT = (((1,), (1,)), ((), ()))
NG = 8
LO, HI = 1, 0
NS = 8
CH = 256
SH = 144
AL = 5
AH = 4
P4HI = (4,) + (3,) * 12
SUB = ((4, 2, 0, 256), (6, 1, 0, 256), (7, 1, 0, 128), (7, 1, 128, 64), (7, 1, 192, 64))
LATE_POS = 1
TOCOL = (8, 9, 10, 11, 6, 7)


def _kernel(x_hbm, k_hbm, v_hbm, wq_hbm, wo_hbm, wr_hbm, wg_hbm, wu_hbm, wd_hbm, out_ref,
            x_v, wr_v, wq_v, k_v, v_v, wo_v, gu_v, wd_v,
            xcol, qacc, guacc, q_s, s_s, m_s, col_s, e_s, ex_s, lsem, hsem, msem, psem):
    hkv, sk = k_hbm.shape[1], k_hbm.shape[2]
    W = k_v.shape[0] * CH
    D = x_v.shape[-1]
    FF = wg_hbm.shape[1]
    rep = HQ // hkv
    HF = FF // 2
    N1, N2, N3, N4 = 16, 2 * W // CH, 2 * W // CH, 16
    BASE = {1: 0, 2: N1, 3: N1 + N2, 4: N1 + N2 + N3}
    NP = {1: N1, 2: N2, 3: N3, 4: N4}
    NWD = FF // 16
    WD_P3 = 4 * (N1 - AH + 2)
    WD_P4 = WD_P3 + 4 * AH
    ST = SH // 8
    assert WD_P4 + sum(P4HI) == NWD and hkv == NG and rep == 4 and D == 4 * DH and N2 + N3 == D // 8
    stream = {1: (wq_hbm, wq_v, 0), 2: (k_hbm.at[0], k_v, sk - W),
              3: (v_hbm.at[0], v_v, sk - W), 4: (wo_hbm, wo_v, 0)}

    def mo(i, m):
        return i if isinstance(i, int) else pl.multiple_of(i, m)

    def low(p, c, t):
        h, v, lo = stream[p]
        gs = pl.ds(4 * t, 4)
        return pltpu.make_async_copy(h.at[gs, pl.ds(mo(lo - SH + c * CH, 16), CH)], v.at[c, gs],
                                     lsem.at[(BASE[p] + 2 * c + t) % NS])

    def low0(p, t, part):
        h, v, lo = stream[p]
        gs = pl.ds(4 * t, 4)
        if part == 0:
            return pltpu.make_async_copy(h.at[gs, pl.ds(lo, CH - SH)], v.at[0, gs, pl.ds(SH, CH - SH)],
                                         lsem.at[(BASE[p] + t) % NS])
        hi = lo + v.shape[0] * CH
        return pltpu.make_async_copy(h.at[gs, pl.ds(hi - SH, SH)], v.at[0, gs, pl.ds(0, SH)],
                                     msem.at[2 + t])

    def go(cp):
        cp.start(priority=LO)

    def wait(cp):
        cp.wait()

    def low_do(p, c, t, act):
        def first():
            act(low0(p, t, 0))
            act(low0(p, t, 1))

        def other():
            act(low(p, c, t))

        if isinstance(c, int):
            (first if c == 0 else other)()
        else:
            pl.when(c == 0)(first)
            pl.when(c > 0)(other)

    def sub(i):
        g0, ng, r0, nr = SUB[i]
        c = N4 // 2 - 1
        return pltpu.make_async_copy(wo_hbm.at[pl.ds(g0, ng), pl.ds(c * CH - SH + r0, nr)],
                                     wo_v.at[c, pl.ds(g0, ng), pl.ds(r0, nr)], msem.at[4 + i])

    def hsem_at(it, k):
        return hsem.at[((it + 2) % NS) * 4 + k]

    def wd_piece(seq):
        return (seq % 2) * (NWD // 2) + seq // 2

    def hi_wd(seq, it, k):
        sl = pl.ds(mo(wd_piece(seq) * 16, 16), 16)
        return pltpu.make_async_copy(wd_hbm.at[sl], wd_v.at[sl], hsem_at(it, k))

    def gu_row(u, k):
        return mo((u // 2 + (k // 2) * (D // 16)) * 8, 8)

    def hi_gu(u, k):
        h = wg_hbm if k % 2 == 0 else wu_hbm
        src = h.at[pl.ds(gu_row(u, k), 8), pl.ds(mo((u % 2) * HF, 128), HF)]
        return pltpu.make_async_copy(src, gu_v.at[u, k], hsem_at(N1 + u - AH, k))

    def branch(cond, fa, fb):
        pl.when(cond)(fa)
        pl.when(jnp.logical_not(cond))(fb)

    def start_low(p, c, t):
        nc = NP[p] // 2
        c2, t2 = c + (t + AL) // 2, (t + AL) % 2
        pl.when(c2 < nc)(lambda: go(low(p, c2, t2)))
        pl.when(c2 == nc)(lambda: low_do(p + 1, 0, t2, go))
        pl.when(c2 > nc)(lambda: go(low(p + 1, c2 - nc, t2)))

    def start_high(p, s, k):
        n, it = NP[p], BASE[p] + s

        def gu():
            hi_gu(it + AH - N1, k).start(priority=HI)

        if p == 1:
            branch(s + AH < n, lambda: hi_wd(4 * (s + 2) + k, it, k).start(priority=HI), gu)
        elif p == 2:
            gu()
        else:
            branch(s + AH < n, gu, lambda: hi_wd(WD_P3 + 4 * (s + AH - n) + k, it, k).start(priority=HI))

    cp_x = pltpu.make_async_copy(x_hbm, x_v, msem.at[0])
    cp_wr = pltpu.make_async_copy(wr_hbm, wr_v, msem.at[1])

    cp_x.start(priority=HI)
    low_do(1, 0, 0, go)
    cp_wr.start(priority=HI)
    for s in range(1, AL):
        low_do(1, s // 2, s % 2, go)

    def pre(j):
        sl = pl.ds(mo(wd_piece(j % 4) * 16 + (j // 4) * 8, 8), 8)
        return pltpu.make_async_copy(wd_hbm.at[sl], wd_v.at[sl], psem.at[j])

    def fill(k, carry):
        pre(k).start(priority=HI)
        d = lax.broadcasted_iota(jnp.int32, (32, D), 0) + k * 32
        p = lax.broadcasted_iota(jnp.int32, (32, D), 1)
        f = p - SH + jnp.where(p < SH, 2 * D, 0)
        e = jnp.where(d == (f // 32) * 8 + f % 8, 1.0, 0.0)
        e_s[pl.ds(pl.multiple_of(k * 32, 32), 32), :] = e.astype(BF16)
        return carry
    lax.fori_loop(0, 8, fill, 0)

    cp_x.wait()
    hi_wd(4, -1, 0).start(priority=HI)
    x = x_v[0].astype(F32)
    mu = jnp.mean(x, axis=-1, keepdims=True)
    xc = x - mu
    qacc[...] = jnp.zeros(qacc.shape, F32)
    guacc[...] = jnp.zeros(guacc.shape, F32)
    cp_wr.wait()
    var = jnp.mean(xc * xc, axis=-1, keepdims=True)
    xn = xc / jnp.sqrt(var + 1e-5)
    pre(0).wait()
    hi_wd(5, -1, 1).start(priority=HI)
    for b in range(D // 128):
        xcol[b * 128:(b + 1) * 128, :] = jnp.transpose(
            jnp.broadcast_to(xn[:, b * 128:(b + 1) * 128], (128, 128)))
        if b % 2 == 1:
            pre(1 + b // 2).wait()
            hi_wd(6 + b // 2, -1, 2 + b // 2).start(priority=HI)
    wr = wr_v[...].astype(F32).reshape(1, D)
    gate = jax.nn.sigmoid(jnp.sum(xn * wr, axis=-1, keepdims=True))

    def lanes(col, n):
        return jnp.concatenate([col] * n, axis=1)

    def p1(c, carry):
        for t in range(2):
            s = 2 * c + t
            low_do(1, c, t, wait)
            for k in range(4):
                @pl.when(s >= AH - 1)
                def _():
                    hi_wd(4 * (s - AH + 2) + k, s - AH, k).wait()
                start_high(1, s, k)
                if k == 0:
                    start_low(1, c, t)
                acc = qacc[8 * k:8 * k + 8]
                for g in range(4 * t, 4 * t + 4):
                    xcur = xcol[pl.ds(pl.multiple_of(g * 64 + c * 8, 8), 8), :]
                    xprv = xcol[pl.ds(pl.multiple_of(g * 64 + ((c + 7) % 8) * 8, 8), 8), :]
                    xs = jnp.concatenate([xprv if tau < ST else xcur for tau in range(8 * k, 8 * k + 8)],
                                         axis=0)
                    acc = acc + (wq_v[c, g, k * 64:(k + 1) * 64, :].astype(F32) * xs).reshape(8, 8, DH)
                qacc[8 * k:8 * k + 8] = acc
        return carry
    lax.fori_loop(0, N1 // 2, p1, 0)
    for j in range(3, 8):
        pre(j).wait()

    row = lax.broadcasted_iota(jnp.int32, (8, DH), 0)
    for h in range(hkv):
        qh = None
        for j in range(rep):
            qn = jnp.sum(qacc[(h * rep + j + ST) % HQ], axis=0, keepdims=True)
            qn = jnp.broadcast_to(qn, (8, DH))
            qh = qn if qh is None else jnp.where(row == j, qn, qh)
        q_s[h] = qh * (DH ** -0.5)

    def ffn_part(u, half, w):
        acc = guacc[w, half]
        for k in (w, w + 2):
            acc = acc + gu_v[u, k].astype(F32) * lanes(xcol[pl.ds(gu_row(u, k), 8), :], HF // 128)
        guacc[w, half] = acc

    def step23(p, c, t, heads):
        s = 2 * c + t
        u = BASE[p] - N1 + s
        low_do(p, c, t, wait)
        start_high(p, s, 0)
        start_low(p, c, t)
        heads(range(4 * t, 4 * t + 2))
        hi_gu(u, 0).wait()
        hi_gu(u, 2).wait()
        start_high(p, s, 1)
        ffn_part(u, t, 0)
        hi_gu(u, 1).wait()
        start_high(p, s, 2)
        heads(range(4 * t + 2, 4 * t + 4))
        hi_gu(u, 3).wait()
        start_high(p, s, 3)
        ffn_part(u, t, 1)

    def p2(c, ms):
        ms = list(ms)

        def heads(hs):
            for h in hs:
                s = lax.dot_general(q_s[h].astype(BF16), k_v[c, h], NT, preferred_element_type=F32)
                s_s[c, h] = s
                ms[h] = jnp.maximum(ms[h], jnp.maximum(s[:, :DH], s[:, DH:]))
        for t in range(2):
            step23(2, c, t, heads)
        return tuple(ms)
    neg = jnp.full((8, DH), -jnp.inf, F32)
    ms = lax.fori_loop(0, N2 // 2, p2, (neg,) * hkv)
    for h in range(hkv):
        m_s[h] = jnp.broadcast_to(jnp.max(ms[h], axis=-1, keepdims=True), (8, DH))

    def p3(c, carry):
        os_, ls = list(carry[0]), list(carry[1])

        def heads(hs):
            for h in hs:
                p = jnp.exp(s_s[c, h] - lanes(m_s[h], 2))
                ls[h] = ls[h] + (p[:, :DH] + p[:, DH:])
                os_[h] = os_[h] + jnp.dot(p.astype(BF16), v_v[c, h], preferred_element_type=F32)
        for t in range(2):
            step23(3, c, t, heads)
        return tuple(os_), tuple(ls)
    zero = jnp.zeros((8, DH), F32)
    os_, ls = lax.fori_loop(0, N3 // 2, p3, ((zero,) * hkv, (zero,) * hkv))

    on = [os_[h] / jnp.sum(ls[h], axis=-1, keepdims=True) for h in range(hkv)]
    both = [jnp.concatenate([o, jnp.concatenate([o[rep - 1:rep], o[:rep - 1], o[rep:]], axis=0)], axis=1)
            for o in on]
    ex_s[...] = jnp.dot(jnp.concatenate(both, axis=0).astype(BF16), e_s[...], preferred_element_type=F32)
    pos = lax.broadcasted_iota(jnp.int32, (8, CH), 1)
    ctmask = lax.broadcasted_iota(jnp.int32, (8, CH), 0) == (pos // 8 + (-ST) % 4) % 4
    g, up = [jnp.concatenate([jnp.sum(guacc[w, hf], axis=0, keepdims=True) for hf in range(2)], axis=1)
             for w in range(2)]
    hid = g * jax.nn.sigmoid(g) * up * gate
    rowf = lax.broadcasted_iota(jnp.int32, (8, FF), 0)
    hb = jnp.where(rowf == 0, hid, 0.0).astype(BF16)

    def to_col(slot, vec):
        col_s[slot * 128:(slot + 1) * 128, :] = jnp.transpose(jnp.broadcast_to(vec, (128, 128)))

    issue = {}
    for j in range(AH):
        for k in range(4):
            issue[WD_P3 + 4 * j + k] = (BASE[4] - AH + j, k)
    pc = WD_P4
    for s, cnt in enumerate(P4HI):
        for k in range(cnt):
            issue[pc] = (BASE[4] + s, k)
            pc += 1
    vblocks = sorted({wd_piece(q) // 8 for q in range(NWD - 16, NWD)})
    assert len(vblocks) == 2
    have = {wd_piece(q) for q in range(WD_P3)}
    waited = set(range(WD_P3))
    todo_blocks = [b for b in range(FF // 128) if b not in vblocks]

    def start_piece(q):
        hi_wd(q, *issue[q]).start(priority=HI)

    def wait_piece(q):
        hi_wd(q, *issue[q]).wait()
        waited.add(q)
        have.add(wd_piece(q))

    def vpu_piece(acc, q):
        p = wd_piece(q)
        if p // 8 not in vblocks:
            return acc
        c0 = (4 + vblocks.index(p // 8)) * 128 + (p % 8) * 16
        prod = wd_v[p * 16:(p + 1) * 16, :].astype(F32) * lanes(col_s[c0:c0 + 16, :], D // 128)
        return acc + jnp.sum(prod.reshape(2, 8, D), axis=0)

    def vpu_wo(acc, gi, r0, nr):
        c = N4 // 2 - 1
        cols = []
        for tau in range(r0 // 8, (r0 + nr) // 8):
            rt = (c * CH // 8 - ST + tau) // 4
            assert rt // 16 == rep - 1
            d0 = (gi - 4) * 128 + (rt % 16) * 8
            cols.append(col_s[d0:d0 + 8, :])
        prod = wo_v[c, gi, r0:r0 + nr, :].astype(F32) * jnp.concatenate(cols, axis=0)
        part = jnp.sum(prod.reshape(nr // 32, 4, 8, DH), axis=0)
        return acc + jnp.concatenate([part[(ct + ST) % 4] for ct in range(4)], axis=1)

    row8 = lax.broadcasted_iota(jnp.int32, (8, D), 0)
    acc = jnp.where(row8 == 0, x + xn, 0.0)
    accw = zero
    for s in range(N4 - 1):
        c, t = s // 2, s % 2
        it = BASE[4] + s
        starts = [q for q, (i, _) in issue.items() if i == it]
        waits = [q for q, (i, _) in issue.items() if i == it - AH]
        l = jnp.concatenate([
            jnp.where(ctmask, ex_s[8 * gi + c // 2:8 * gi + c // 2 + 1, (c % 2) * CH:(c % 2 + 1) * CH], 0.0)
            for gi in range(4 * t, 4 * t + 4)], axis=1).astype(BF16)
        low_do(4, c, t, wait)
        for q in starts[:1]:
            start_piece(q)
        if s + AL < N4 - 1:
            low_do(4, (s + AL) // 2, (s + AL) % 2, go)
        elif s + AL == N4 - 1:
            for i in range(len(SUB)):
                go(sub(i))
        accw = accw + jnp.dot(l, wo_v[c, 4 * t:4 * t + 4].reshape(4 * CH, DH), preferred_element_type=F32)
        for q in waits[:-1]:
            wait_piece(q)
        for q in starts[1:2]:
            start_piece(q)
        ready = [b for b in todo_blocks if all(p in have for p in range(8 * b, 8 * b + 8))]
        for b in ready[:1]:
            todo_blocks.remove(b)
            acc = acc + jnp.dot(hb[:, b * 128:(b + 1) * 128], wd_v[b * 128:(b + 1) * 128, :],
                                preferred_element_type=F32)
        for slot in range(6):
            if TOCOL[slot] == s:
                if slot < 4:
                    to_col(slot, on[4 + slot][rep - 1:rep, :])
                else:
                    b = vblocks[slot - 4]
                    to_col(slot, hid[:, b * 128:(b + 1) * 128])
        for q in waits[-1:]:
            wait_piece(q)
        for q in starts[2:3]:
            start_piece(q)
        for q in waits:
            assert wd_piece(q) // 8 not in vblocks or s > max(TOCOL[4:])
            acc = vpu_piece(acc, q)
        for q in starts[3:]:
            start_piece(q)
    assert not todo_blocks
    acc = acc + jnp.concatenate([jnp.where(row == ct, accw, 0.0) for ct in range(4)], axis=1)
    rest = [q for q in range(NWD) if q not in waited]
    last_it = max(issue[q][0] for q in rest)
    for q in rest:
        if issue[q][0] != last_it:
            wait_piece(q)
            acc = vpu_piece(acc, q)
    for i in range(len(SUB)):
        if i == LATE_POS:
            late = [q for q in rest if issue[q][0] == last_it]
            for q in late:
                wait_piece(q)
            for q in late:
                acc = vpu_piece(acc, q)
        g0, ng, r0, nr = SUB[i]
        sub(i).wait()
        for gi in range(g0, g0 + ng):
            acc = vpu_wo(acc, gi, r0, nr)
    out_ref[0] = jnp.sum(acc, axis=0, keepdims=True).astype(out_ref.dtype)


def _tiles(w):
    r, c = w.shape
    return w.reshape(r // 8, 8, c // 128, 128).transpose(0, 2, 1, 3).reshape(NG, -1, 128)


@jax.jit
def pallas_parallel_sum__sliding_block_cached__moe_arch_mod__decode_kernel(
    A_x: jax.Array,
    A_k_cache: jax.Array,
    A_v_cache: jax.Array,
    A_wq: jax.Array,
    A_wo: jax.Array,
    B_x: jax.Array,
    B_w_r: jax.Array,
    B_w_gate: jax.Array,
    B_w_up: jax.Array,
    B_w_down: jax.Array,
):
    del B_x
    hkv, sk = A_k_cache.shape[1], A_k_cache.shape[2]
    W = min(4096, max(256, sk // 4))
    D = A_x.shape[-1]
    FF = B_w_gate.shape[1]
    nkc = W // CH
    anyspec = pl.BlockSpec(memory_space=pl.ANY)
    return pl.pallas_call(
        _kernel,
        out_shape=jax.ShapeDtypeStruct(A_x.shape, A_x.dtype),
        in_specs=[anyspec] * 9,
        out_specs=pl.BlockSpec(memory_space=pltpu.VMEM),
        scratch_shapes=[
            pltpu.VMEM(A_x.shape, BF16), pltpu.VMEM(B_w_r.shape, BF16),
            pltpu.VMEM((8, NG, CH, DH), BF16),
            pltpu.VMEM((nkc, hkv, CH, DH), BF16), pltpu.VMEM((nkc, hkv, CH, DH), BF16),
            pltpu.VMEM((8, NG, CH, DH), BF16),
            pltpu.VMEM((4 * nkc, 4, 8, FF // 2), BF16), pltpu.VMEM(B_w_down.shape, BF16),
            pltpu.VMEM((D, 128), F32), pltpu.VMEM((HQ, 8, DH), F32), pltpu.VMEM((2, 2, 8, FF // 2), F32),
            pltpu.VMEM((hkv, 8, DH), F32), pltpu.VMEM((nkc, hkv, 8, CH), F32),
            pltpu.VMEM((hkv, 8, DH), F32),
            pltpu.VMEM((6 * 128, 128), F32), pltpu.VMEM((2 * DH, D), BF16), pltpu.VMEM((8 * hkv, D), F32),
            pltpu.SemaphoreType.DMA((NS,)), pltpu.SemaphoreType.DMA((NS * 4,)),
            pltpu.SemaphoreType.DMA((4 + len(SUB),)), pltpu.SemaphoreType.DMA((8,)),
        ],
        compiler_params=pltpu.CompilerParams(
            vmem_limit_bytes=48 * 1024 * 1024,
            disable_semaphore_checks=True,
        ),
    )(A_x, A_k_cache, A_v_cache, _tiles(A_wq), _tiles(A_wo), B_w_r, B_w_gate, B_w_up, B_w_down)
```
